```python
import jax
import jax.numpy as jnp

def _softmax(x, axis=-1):
    return jax.nn.softmax(x, axis=axis)
def _gelu(x):
    return jax.nn.gelu(x, approximate=True)
def _silu(x):
    return jax.nn.silu(x)
def _sigmoid(x):
    return jax.nn.sigmoid(x)
def _layernorm(x, axis=-1, eps=1e-5):
    m = jnp.mean(x, axis=axis, keepdims=True)
    v = jnp.var(x, axis=axis, keepdims=True)
    return (x - m) / jnp.sqrt(v + eps)
def _scatter_add(tgt, idx, src, axis=0):
    return tgt.at[idx].add(src)
def _segment_sum(src, seg, n):
    return jax.ops.segment_sum(src, seg, n)
class _Rng:
    def __init__(self, key):
        self._k = key
    def _next(self):
        self._k, sub = jax.random.split(self._k)
        return sub
    def normal(self, shape):
        return jax.random.normal(self._next(), shape, dtype=jnp.bfloat16)
    def randint(self, lo, hi, shape):
        return jax.random.randint(self._next(), shape, lo, hi, dtype=jnp.int32)
    def uniform(self, shape, lo=0.0, hi=1.0):
        return jax.random.uniform(self._next(), shape, jnp.bfloat16, lo, hi)
    def permutation(self, n):
        return jax.random.permutation(self._next(), n)


kernel_name = 'sequential_preLN__sliding_block_cached__mixer_s_mlp__decode'

def setup_inputs():
    _rng = _Rng(jax.random.key(int.from_bytes(__import__("os").urandom(4), "little")))
    _w = (lambda a: (lambda t: t.astype(jnp.bfloat16) if jnp.issubdtype(t.dtype, jnp.floating) else t)(jnp.asarray(a)))
    def _A_setup():
        B, Sq, D = 1, 1, 640
        Hq, Hkv, Sk, Dh = 32, 32, 32768, 192
        assert Hq % Hkv == 0, (Hq, Hkv)
        return {
            "x": _w((lambda *s: _rng.normal(s) * 0.05)(B, Sq, D)),
            "k_cache": _w((lambda *s: _rng.normal(s) * 0.05)(B, Hkv, Sk, Dh)),
            "v_cache": _w((lambda *s: _rng.normal(s) * 0.05)(B, Hkv, Sk, Dh)),
            "wq": _w((lambda *s: _rng.normal(s) * 0.05)(D, Hq * Dh) * (D ** -0.5)),
            "wo": _w((lambda *s: _rng.normal(s) * 0.05)(Hq * Dh, D) * ((Hq * Dh) ** -0.5)),
        }
    _A_in = _A_setup()

    def _B_setup():
        B, S, D, F = 1, 1, 640, 1536
        return {
            "x":  _w((lambda *s: _rng.normal(s) * 0.05)(B, S, D)),
            "w1": _w((lambda *s: _rng.normal(s) * 0.05)(D, D) * (D ** -0.5)),
            "w2": _w((lambda *s: _rng.normal(s) * 0.05)(D, D) * (D ** -0.5)),
            "w3": _w((lambda *s: _rng.normal(s) * 0.05)(D, F) * (D ** -0.5)),
            "w4": _w((lambda *s: _rng.normal(s) * 0.05)(F, D) * (F ** -0.5)),
        }
    _B_in = _B_setup()

    return {
        "A_x": _A_in["x"],
        "A_k_cache": _A_in["k_cache"],
        "A_v_cache": _A_in["v_cache"],
        "A_wq": _A_in["wq"],
        "A_wo": _A_in["wo"],
        "B_x": _B_in["x"],
        "B_w1": _B_in["w1"],
        "B_w2": _B_in["w2"],
        "B_w3": _B_in["w3"],
        "B_w4": _B_in["w4"],
    }

def reference(A_x, A_k_cache, A_v_cache, A_wq, A_wo, B_x, B_w1, B_w2, B_w3, B_w4):
    def _A_ref(x, k_cache, v_cache, wq, wo):
        B, Sq, D = x.shape
        Hq, Dh = 32, 192
        Hkv, Sk = k_cache.shape[1], k_cache.shape[2]
        W = min(4096, max(256, Sk // 4))
        rep = Hq // Hkv
        q = (lambda x, *d: x.transpose(*d))((x @ wq).reshape(B, Sq, Hq, Dh), 0, 2, 1, 3)
        k = jnp.repeat(k_cache[:, :, Sk - W:, :], rep, axis=1)
        v = jnp.repeat(v_cache[:, :, Sk - W:, :], rep, axis=1)
        scores = jnp.einsum("bhqd,bhkd->bhqk", q, k) * (Dh ** -0.5)
        p = _softmax(scores, axis=-1)
        o = jnp.einsum("bhqk,bhkd->bhqd", p, v)
        return (lambda x, *d: x.transpose(*d))(o, 0, 2, 1, 3).reshape(B, Sq, Hq * Dh) @ wo

    def _B_ref(x, w1, w2, w3, w4):
        B, S, D = x.shape
        h = _gelu(_layernorm(x, axis=-1) @ w1)
        c = D // 4
        g0 = jnp.pad(h[:, :, 0*c:1*c], ((0, 0), (1, 0), (0, 0)))[:, :S, :]
        g1 = jnp.pad(h[:, :, 1*c:2*c], ((0, 0), (0, 1), (0, 0)))[:, 1:, :]
        g2 = jnp.pad(h[:, :, 2*c:3*c], ((0, 0), (2, 0), (0, 0)))[:, :S, :]
        g3 = jnp.pad(h[:, :, 3*c:   ], ((0, 0), (0, 2), (0, 0)))[:, 2:, :]
        hs = jnp.concatenate([g0, g1, g2, g3], axis=-1) @ w2
        x1 = x + hs
        h2 = _gelu(_layernorm(x1, axis=-1) @ w3) @ w4
        return x1 + h2

    x = A_x
    h = x + _A_ref(_layernorm(x, axis=-1), A_k_cache, A_v_cache, A_wq, A_wo)
    h2 = h + _B_ref(_layernorm(h, axis=-1), B_w1, B_w2, B_w3, B_w4)
    return h2
```

```python
import functools

import jax
import jax.numpy as jnp
from jax import lax
import jax.experimental.pallas as pl
import jax.experimental.pallas.tpu as pltpu

_F32 = jnp.float32
_BF16 = jnp.bfloat16
_LANES = 128
_EPS = 1e-5


def _layernorm(x):
    m = jnp.mean(x, axis=-1, keepdims=True)
    c = x - m
    v = jnp.mean(c * c, axis=-1, keepdims=True)
    return c / jnp.sqrt(v + _EPS)


def _kernel(x_hbm, k_hbm, v_hbm, wq_hbm, wo_hbm, w3_hbm, w4_hbm, out_ref,
            xbuf, wqbuf, kbuf, vbuf, wobuf, w3buf, w4buf, qcol, ocol,
            sem_x, sem_wq, sem_k, sem_v, sem_wo, sem_w3, sem_w4,
            *, H, DH, SK, W, D, F, NB, NQ, NO, N3, N4, CH):
    HD = H * DH
    qc_w = HD // NQ
    oc_r = HD // NO
    c3 = F // N3
    r4 = F // N4

    x_cp = pltpu.make_async_copy(x_hbm, xbuf, sem_x.at[0])

    def wq_cp(c):
        return pltpu.make_async_copy(wq_hbm.at[:, pl.ds(c * qc_w, qc_w)],
                                     wqbuf.at[:, pl.ds(c * qc_w, qc_w)], sem_wq.at[c])

    def k_cp(h, slot):
        return pltpu.make_async_copy(k_hbm.at[h, :, pl.ds(SK - W, W)], kbuf.at[slot], sem_k.at[slot])

    def v_cp(h, slot):
        return pltpu.make_async_copy(v_hbm.at[h, :, pl.ds(SK - W, W)], vbuf.at[slot], sem_v.at[slot])

    def wo_cp(c):
        return pltpu.make_async_copy(wo_hbm.at[pl.ds(c * oc_r, oc_r), :],
                                     wobuf.at[pl.ds(c * oc_r, oc_r), :], sem_wo.at[c])

    def w3_cp(c):
        return pltpu.make_async_copy(w3_hbm.at[:, pl.ds(c * c3, c3)],
                                     w3buf.at[:, pl.ds(c * c3, c3)], sem_w3.at[c])

    def w4_cp(c):
        return pltpu.make_async_copy(w4_hbm.at[pl.ds(c * r4, r4), :],
                                     w4buf.at[pl.ds(c * r4, r4), :], sem_w4.at[c])

    x_cp.start()
    for c in range(NQ):
        wq_cp(c).start()
    for h in range(NB):
        k_cp(h, h).start()
        v_cp(h, h).start()

    x_cp.wait()
    x = xbuf[...].astype(_F32)
    xn = jnp.broadcast_to(_layernorm(x).astype(_BF16), (8, D))
    scale = DH ** -0.5
    for c in range(NQ):
        wq_cp(c).wait()
        q = jnp.dot(xn, wqbuf[:, c * qc_w:(c + 1) * qc_w], preferred_element_type=_F32)
        q = q[0:1, :].astype(_BF16).astype(_F32) * scale
        for j in range(qc_w // _LANES):
            blk = jnp.broadcast_to(q[:, j * _LANES:(j + 1) * _LANES], (_LANES, _LANES))
            qcol[c * qc_w + j * _LANES:c * qc_w + (j + 1) * _LANES, :] = blk.T

    rep = CH // _LANES

    def head(h, carry):
        slot = h % NB
        row0 = pl.multiple_of(h * DH, 8)
        qc = qcol[pl.ds(row0, DH), :]
        qc = jnp.concatenate([qc] * rep, axis=1)
        k_cp(h, slot).wait()
        parts = []
        for c in range(W // CH):
            kf = kbuf[slot, :, c * CH:(c + 1) * CH].astype(_F32)
            parts.append(jnp.sum(kf * qc, axis=0, keepdims=True))
        s = jnp.concatenate(parts, axis=1)

        @pl.when(h + NB < H)
        def _():
            k_cp(h + NB, slot).start()

        m = jnp.max(s, axis=1, keepdims=True)
        p = jnp.exp(s - m)
        l = jnp.sum(p, axis=1, keepdims=True)
        v_cp(h, slot).wait()
        acc = jnp.zeros((DH, _LANES), _F32)
        for c in range(W // CH):
            vf = vbuf[slot, :, c * CH:(c + 1) * CH].astype(_F32)
            pv = vf * p[:, c * CH:(c + 1) * CH]
            for r in range(rep):
                acc = acc + pv[:, r * _LANES:(r + 1) * _LANES]

        @pl.when(h + NB < H)
        def _():
            v_cp(h + NB, slot).start()

        @pl.when(h + NB == H - 1)
        def _():
            for c in range(NO):
                wo_cp(c).start()
            for c in range(N3):
                w3_cp(c).start()
            for c in range(N4):
                w4_cp(c).start()

        o = jnp.sum(acc, axis=1, keepdims=True) / l
        ocol[pl.ds(row0, DH), :] = jnp.broadcast_to(o, (DH, _LANES))
        return carry

    lax.fori_loop(0, H, head, 0)

    RB = 64
    att = jnp.zeros((8, D), _F32)
    for c in range(NO):
        wo_cp(c).wait()

        def wo_body(i, a, c=c):
            r0 = pl.multiple_of(c * oc_r + i * RB, RB)
            oc = ocol[pl.ds(r0, RB), :]
            oc = jnp.concatenate([oc] * (D // _LANES), axis=1)
            wf = wobuf[pl.ds(r0, RB), :].astype(_F32)
            return a + jnp.sum((wf * oc).reshape(RB // 8, 8, D), axis=0)

        att = lax.fori_loop(0, oc_r // RB, wo_body, att)
    hres = x + jnp.sum(att, axis=0, keepdims=True)

    x1 = _layernorm(hres)
    y = jnp.broadcast_to(_layernorm(x1).astype(_BF16), (8, D))
    hid = []
    for c in range(N3):
        w3_cp(c).wait()
        t = jnp.dot(y, w3buf[:, c * c3:(c + 1) * c3], preferred_element_type=_F32)
        hid.append(jax.nn.gelu(t, approximate=True).astype(_BF16))
    hid = jnp.concatenate(hid, axis=1)
    mlp = jnp.zeros((8, D), _F32)
    for c in range(N4):
        w4_cp(c).wait()
        mlp = mlp + jnp.dot(hid[:, c * r4:(c + 1) * r4], w4buf[c * r4:(c + 1) * r4, :],
                            preferred_element_type=_F32)
    out_ref[...] = (hres + (x1 + mlp[0:1, :])).astype(out_ref.dtype)


def _build(A_x, A_k_cache, A_v_cache, A_wq, A_wo, B_w3, B_w4, *, NB=3, NQ=4, NO=4, N3=4, N4=4, CH=256):
    B, S, D = A_x.shape
    _, H, SK, DH = A_k_cache.shape
    assert B == 1 and S == 1
    W = min(4096, max(256, SK // 4))
    F = B_w3.shape[1]
    HD = H * DH
    kt = jnp.swapaxes(A_k_cache[0], 1, 2)
    vt = jnp.swapaxes(A_v_cache[0], 1, 2)
    x2 = A_x.reshape(1, D)
    kern = functools.partial(_kernel, H=H, DH=DH, SK=SK, W=W, D=D, F=F,
                             NB=NB, NQ=NQ, NO=NO, N3=N3, N4=N4, CH=CH)
    dma = pltpu.SemaphoreType.DMA
    out = pl.pallas_call(
        kern,
        out_shape=jax.ShapeDtypeStruct((1, D), A_x.dtype),
        in_specs=[pl.BlockSpec(memory_space=pl.ANY)] * 7,
        out_specs=pl.BlockSpec(memory_space=pltpu.VMEM),
        scratch_shapes=[
            pltpu.VMEM((1, D), A_x.dtype),
            pltpu.VMEM((D, HD), A_wq.dtype),
            pltpu.VMEM((NB, DH, W), A_k_cache.dtype),
            pltpu.VMEM((NB, DH, W), A_v_cache.dtype),
            pltpu.VMEM((HD, D), A_wo.dtype),
            pltpu.VMEM((D, F), B_w3.dtype),
            pltpu.VMEM((F, D), B_w4.dtype),
            pltpu.VMEM((HD, _LANES), _F32),
            pltpu.VMEM((HD, _LANES), _F32),
            dma((1,)), dma((NQ,)), dma((NB,)), dma((NB,)), dma((NO,)), dma((N3,)), dma((N4,)),
        ],
        compiler_params=pltpu.CompilerParams(vmem_limit_bytes=96 * 1024 * 1024),
    )(x2, kt, vt, A_wq, A_wo, B_w3, B_w4)
    return out.reshape(B, S, D)


@jax.jit
def pallas_sequential_preLN__sliding_block_cached__mixer_s_mlp__decode_kernel(
    A_x: jax.Array,
    A_k_cache: jax.Array,
    A_v_cache: jax.Array,
    A_wq: jax.Array,
    A_wo: jax.Array,
    B_x: jax.Array,
    B_w1: jax.Array,
    B_w2: jax.Array,
    B_w3: jax.Array,
    B_w4: jax.Array,
):
    return _build(A_x, A_k_cache, A_v_cache, A_wq, A_wo, B_w3, B_w4)
```

```python
import functools

import jax
import jax.numpy as jnp
from jax import lax
import jax.experimental.pallas as pl
import jax.experimental.pallas.tpu as pltpu

_F32 = jnp.float32
_BF16 = jnp.bfloat16
_L = 128
_EPS = 1e-5
_RING = 32


def _layernorm(x):
    m = jnp.mean(x, axis=-1, keepdims=True)
    c = x - m
    v = jnp.mean(c * c, axis=-1, keepdims=True)
    return c / jnp.sqrt(v + _EPS)


def _perm(items, k):
    m = len(items) // k
    return [items[(i % k) * m + i // k] for i in range(len(items))]


class _Stream:
    def __init__(self, sems, priority, phase):
        self.sems, self.priority, self.n = sems, priority, phase
        self.pending = {}

    def adopt(self, slot, key, src, dst):
        self.pending[slot] = (key, pltpu.make_async_copy(src, dst, self.sems.at[slot]))

    def ensure(self, key):
        for slot, (k, cp) in list(self.pending.items()):
            if k == key:
                cp.wait()
                del self.pending[slot]

    def wait_slot(self, slot):
        if slot in self.pending:
            self.pending.pop(slot)[1].wait()

    def start(self, key, src, dst):
        slot = self.n % _RING
        self.n += 1
        self.wait_slot(slot)
        cp = pltpu.make_async_copy(src, dst, self.sems.at[slot])
        cp.start(priority=self.priority)
        self.pending[slot] = (key, cp)

    def drain(self):
        for slot in list(self.pending):
            self.wait_slot(slot)


def _kernel(x_hbm, k_hbm, v_hbm, wq_hbm, wo_hbm, w3_hbm, w4_hbm, out_ref,
            xbuf, wqbuf, kbuf, vbuf, wobuf, w3buf, w4buf, qcol, slow, ssum, pb, attbuf,
            sem_a, sem_b, *, H, DH, SK, W, D, F, DA, QSP, DA4, W4G):
    HD = H * DH
    PR = DH // 2
    NC = W // _L
    assert NC == _RING
    c0 = SK - W
    G = PR // 8

    def kv_piece(hbm, buf, row0, half, c):
        return hbm.at[pl.ds(row0, PR), pl.ds(c0 + c * _L, _L)], buf.at[half, c]

    def qk(half, c, q):
        kf = kbuf[half, c].astype(_F32)
        return jnp.sum((kf * q).reshape(G, 8, _L), axis=0)

    def pv(half, c, par, acc):
        vf = vbuf[half, c].astype(_F32)
        p = pb[par, c]
        return acc + (vf.reshape(G, 8, _L) * p[None]).reshape(PR, _L)

    def softmax_p():
        s = ssum[pl.ds(0, NC, stride=8), :]
        for r in range(1, 8):
            s = s + ssum[pl.ds(r, NC, stride=8), :]
        m = jnp.max(jnp.max(s, axis=0, keepdims=True), axis=1, keepdims=True)
        e = jnp.exp(s - m)
        l = jnp.sum(jnp.sum(e, axis=0, keepdims=True), axis=1, keepdims=True)
        return e / l

    def store_p(p, par, c):
        pb[par, c] = jnp.broadcast_to(p[c:c + 1, :], (8, _L))

    def wo_mac(osum, g, row0, att):
        oc = jnp.broadcast_to(osum[g * 8:(g + 1) * 8, :], (8, D))
        wf = wobuf[pl.ds(row0 + g * 8, 8), :].astype(_F32)
        return att + wf * oc

    def half_slot(half, *, step, q=None, par=None, prev=None, att=None, do_softmax=None, extra=None):
        acc = jnp.zeros((PR, _L), _F32) if par is not None else None
        osum = None
        p_new = None
        for c in range(NC):
            step(c)
            if c == 0 and prev is not None:
                osum = jnp.sum(prev[0], axis=1, keepdims=True)
            if c == 0 and do_softmax is not None:
                p_new = softmax_p()
            if q is not None:
                part = qk(1 - half, c, q)
                if half == 0:
                    ssum[c * 8:(c + 1) * 8, :] = part + slow[c]
                else:
                    slow[c] = part
            if par is not None:
                acc = pv(half, c, par, acc)
            if prev is not None and 4 <= c < 4 + G:
                att = wo_mac(osum, c - 4, prev[1], att)
            if p_new is not None and 8 <= c < 24:
                store_p(p_new, do_softmax, 2 * (c - 8))
                store_p(p_new, do_softmax, 2 * (c - 8) + 1)
            if extra is not None:
                extra(c)
        return acc, att

    QC = 1536
    wq_p = _perm([(("wq",), wq_hbm.at[pl.ds(r, 8), pl.ds(c, QC)], wqbuf.at[pl.ds(r, 8), pl.ds(c, QC)])
                  for r in range(0, D, 8) for c in range(0, HD, QC)], 16)
    OR = 24
    wo_p = _perm([(("wo",), wo_hbm.at[pl.ds(r, OR), :], wobuf.at[pl.ds(r, OR), :])
                  for r in range(0, HD, OR)], 16)
    k_pre = [(("k", hh, c),) + kv_piece(k_hbm, kbuf, hh * PR, hh % 2, c) for hh in range(4) for c in range(NC)]
    v_pre = [(("v", 0, c),) + kv_piece(v_hbm, vbuf, 0, 0, c) for c in range(NC)]
    n_w = len(wq_p) + len(wo_p)
    T0 = (n_w + len(k_pre) - DA + 1) // 2
    n_wa = n_w - T0
    allw = wq_p + wo_p
    a_w = allw[0:2 * n_wa:2]
    b_w = allw[1:2 * n_wa:2] + allw[2 * n_wa:]
    assert len(b_w) == T0
    a_list = [(("x",), x_hbm, xbuf)] + a_w + k_pre
    b_list = b_w + v_pre
    up_a = len(a_list) - T0
    A = _Stream(sem_a, 0, (-len(a_list)) % _RING)
    B = _Stream(sem_b, 1, (-len(b_list)) % _RING)
    for pc in a_list[:up_a]:
        A.start(*pc)
    for pc in b_list[:_RING]:
        B.start(*pc)

    A.ensure(("x",))
    x = xbuf[...].astype(_F32)
    xn = jnp.broadcast_to(_layernorm(x).astype(_BF16), (8, D))
    scale = DH ** -0.5

    def pre_step(t):
        B.start(*b_list[t + _RING])
        A.start(*a_list[up_a + t])

    QG = 4 * _L
    ng = HD // QG
    q_rowvals = {}

    def qproj(g):
        if g < ng:
            q = jnp.dot(xn, wqbuf[:, g * QG:(g + 1) * QG], preferred_element_type=_F32)
            q_rowvals[g] = q[0:1, :].astype(_BF16).astype(_F32) * scale
        if g > 0:
            q = q_rowvals.pop(g - 1)
            for j in range(QG // _L):
                r = (g - 1) * QG + j * _L
                qcol[r:r + _L, :] = jnp.broadcast_to(q[:, j * _L:(j + 1) * _L], (_L, _L)).T

    t_q = len(wq_p) // 2 + 2
    t_k = T0 - 4 * NC
    q_sched = {t_q + g * QSP: g for g in range(ng + 1)}
    assert t_q + QSP < t_k + NC and t_q + ng * QSP < T0

    def q_extra(t):
        if t in q_sched:
            A.ensure(("wq",))
            B.ensure(("wq",))
            qproj(q_sched[t])

    for t in range(t_k):
        pre_step(t)
        q_extra(t)

    def q_rows(row0):
        return qcol[pl.ds(row0, PR), :]

    half_slot(0, step=lambda c: pre_step(t_k + c), extra=lambda c: q_extra(t_k + c))
    half_slot(1, step=lambda c: pre_step(t_k + NC + c), q=q_rows(0), extra=lambda c: q_extra(t_k + NC + c))
    half_slot(0, step=lambda c: pre_step(t_k + 2 * NC + c), q=q_rows(PR), extra=lambda c: q_extra(t_k + 2 * NC + c))
    half_slot(1, step=lambda c: pre_step(t_k + 3 * NC + c), q=q_rows(2 * PR), do_softmax=0,
              extra=lambda c: q_extra(t_k + 3 * NC + c))
    A.pending.clear()
    B.pending.clear()

    def loop_step(j, half):
        r_v = pl.multiple_of(j * DH + (half + 1) * PR, 8)
        r_k = pl.multiple_of((j + 2) * DH + half * PR, 8)

        def step(c):
            pltpu.make_async_copy(*kv_piece(v_hbm, vbuf, 0, half, c), sem_b.at[c]).wait()
            pltpu.make_async_copy(*kv_piece(k_hbm, kbuf, 0, 1 - half, c), sem_a.at[c]).wait()
            pltpu.make_async_copy(*kv_piece(k_hbm, kbuf, r_k, half, c), sem_a.at[c]).start(priority=0)
            pltpu.make_async_copy(*kv_piece(v_hbm, vbuf, r_v, 1 - half, c), sem_b.at[c]).start(priority=1)
        return step

    def body(j, carry):
        acc_prev, att = carry
        par = j & 1
        r0 = pl.multiple_of(j * DH, 8)
        r_prev = pl.multiple_of(jnp.maximum(r0 - PR, 0), 8)
        acc, att = half_slot(0, step=loop_step(j, 0), q=q_rows(r0 + DH + PR), par=par,
                             prev=(acc_prev, r_prev), att=att)
        acc, att = half_slot(1, step=loop_step(j, 1), q=q_rows(r0 + 2 * DH), par=par,
                             prev=(acc, r0), att=att, do_softmax=1 - par)
        return acc, att

    NL = H - 2
    acc, att = lax.fori_loop(0, NL, body, (jnp.zeros((PR, _L), _F32), jnp.zeros((8, D), _F32)))

    A = _Stream(sem_a, 0, 0)
    B = _Stream(sem_b, 1, 0)
    for c in range(NC):
        A.adopt(c, ("k", c), *kv_piece(k_hbm, kbuf, 0, 1, c))
        B.adopt(c, ("v", c), *kv_piece(v_hbm, vbuf, 0, 0, c))
    w3_p = _perm([(("w3",), w3_hbm.at[pl.ds(r, 8), :], w3buf.at[pl.ds(r, 8), :]) for r in range(0, D, 8)], 4)
    w4_p = [(("w4", r, n), w4_hbm.at[pl.ds(r * _L, _L), pl.ds(n * _L, _L)], w4buf.at[n, pl.ds(r * _L, _L), :])
            for r in range(F // _L) for n in range(D // _L)]
    w4_b = w4_p[0::2]
    w4_a = w4_p[1::2]
    b_post = [(("v", hh, c),) + kv_piece(v_hbm, vbuf, hh * PR, hh % 2, c)
              for hh in range(2 * NL + 1, 2 * H) for c in range(NC)] + w4_b
    n_post = 4 * NC
    a_sched = {}
    for i, pc in enumerate(w3_p):
        a_sched[(i * (n_post - DA4)) // len(w3_p)] = pc
    for i, pc in enumerate(w4_a[:DA4]):
        a_sched[n_post - DA4 + i] = pc

    def post_step(t):
        slot = t % _RING
        if t < len(b_post):
            B.start(*b_post[t])
        else:
            B.wait_slot(slot)
        if t < NC:
            A.ensure(("k", t))
        if t in a_sched:
            A.start(*a_sched[t])

    r30 = NL * DH
    acc, att = half_slot(0, step=lambda c: post_step(c), q=q_rows(r30 + DH + PR), par=NL & 1,
                         prev=(acc, r30 - PR), att=att)
    acc, att = half_slot(1, step=lambda c: post_step(NC + c), par=NL & 1,
                         prev=(acc, r30), att=att, do_softmax=1 - (NL & 1))
    acc, att = half_slot(0, step=lambda c: post_step(2 * NC + c), par=1 - (NL & 1),
                         prev=(acc, r30 + PR), att=att)
    acc, att = half_slot(1, step=lambda c: post_step(3 * NC + c), par=1 - (NL & 1),
                         prev=(acc, r30 + DH), att=att)

    rest_a = list(w4_a[DA4:])

    def pace(n):
        for _ in range(n):
            if rest_a:
                A.start(*rest_a.pop(0))

    osum = jnp.sum(acc, axis=1, keepdims=True)
    for g in range(G):
        att = wo_mac(osum, g, r30 + DH + PR, att)
    pace(2)
    hres = x + jnp.sum(att, axis=0, keepdims=True)
    x1 = _layernorm(hres)
    pace(3)
    y = jnp.broadcast_to(_layernorm(x1).astype(_BF16), (8, D))
    pace(3)
    A.ensure(("w3",))
    hid = []
    C3 = 384
    for c in range(F // C3):
        tt = jnp.dot(y, w3buf[:, c * C3:(c + 1) * C3], preferred_element_type=_F32)
        hid.append(jax.nn.gelu(tt, approximate=True).astype(_BF16))
        B.ensure(w4_b[c][0])
        pace(3 if c < F // C3 - 1 else 99)
    hid = jnp.concatenate(hid, axis=1)
    mlp = [jnp.zeros((8, _L), _F32) for _ in range(D // _L)]
    lo = 0
    for hi in W4G:
        for key, _, _ in w4_p[lo:hi]:
            A.ensure(key)
            B.ensure(key)
        for key, _, _ in w4_p[lo:hi]:
            _, r, n = key
            mlp[n] = mlp[n] + jnp.dot(hid[:, r * _L:(r + 1) * _L], w4buf[n, r * _L:(r + 1) * _L, :],
                                      preferred_element_type=_F32)
        lo = hi
    A.drain()
    B.drain()
    mlp = jnp.concatenate(mlp, axis=1)
    out_ref[...] = (hres + (x1 + mlp[0:1, :])).astype(out_ref.dtype)


def _build(A_x, A_k_cache, A_v_cache, A_wq, A_wo, B_w3, B_w4, *, DA=12, QSP=13, DA4=8, W4G=(30, 45, 55, 60)):
    B, S, D = A_x.shape
    _, H, SK, DH = A_k_cache.shape
    assert B == 1 and S == 1
    W = min(4096, max(256, SK // 4))
    F = B_w3.shape[1]
    HD = H * DH
    PR = DH // 2
    NC = W // _L
    kt = jnp.swapaxes(A_k_cache[0], 1, 2).reshape(HD, SK)
    vt = jnp.swapaxes(A_v_cache[0], 1, 2).reshape(HD, SK)
    x2 = A_x.reshape(1, D)
    kern = functools.partial(_kernel, H=H, DH=DH, SK=SK, W=W, D=D, F=F, DA=DA, QSP=QSP, DA4=DA4, W4G=W4G)
    dma = pltpu.SemaphoreType.DMA
    out = pl.pallas_call(
        kern,
        out_shape=jax.ShapeDtypeStruct((1, D), A_x.dtype),
        in_specs=[pl.BlockSpec(memory_space=pl.ANY)] * 7,
        out_specs=pl.BlockSpec(memory_space=pltpu.VMEM),
        scratch_shapes=[
            pltpu.VMEM((1, D), A_x.dtype),
            pltpu.VMEM((D, HD), A_wq.dtype),
            pltpu.VMEM((2, NC, PR, _L), A_k_cache.dtype),
            pltpu.VMEM((2, NC, PR, _L), A_v_cache.dtype),
            pltpu.VMEM((HD, D), A_wo.dtype),
            pltpu.VMEM((D, F), B_w3.dtype),
            pltpu.VMEM((D // _L, F, _L), B_w4.dtype),
            pltpu.VMEM((HD, _L), _F32),
            pltpu.VMEM((NC, 8, _L), _F32),
            pltpu.VMEM((NC * 8, _L), _F32),
            pltpu.VMEM((2, NC, 8, _L), _F32),
            pltpu.VMEM((8, D), _F32),
            dma((_RING,)), dma((_RING,)),
        ],
        compiler_params=pltpu.CompilerParams(
            vmem_limit_bytes=64 * 1024 * 1024,
            disable_bounds_checks=True,
            disable_semaphore_checks=True,
        ),
    )(x2, kt, vt, A_wq, A_wo, B_w3, B_w4)
    return out.reshape(B, S, D)


@jax.jit
def pallas_sequential_preLN__sliding_block_cached__mixer_s_mlp__decode_kernel(
    A_x: jax.Array,
    A_k_cache: jax.Array,
    A_v_cache: jax.Array,
    A_wq: jax.Array,
    A_wo: jax.Array,
    B_x: jax.Array,
    B_w1: jax.Array,
    B_w2: jax.Array,
    B_w3: jax.Array,
    B_w4: jax.Array,
):
    return _build(A_x, A_k_cache, A_v_cache, A_wq, A_wo, B_w3, B_w4)
```

```python
import functools

import jax
import jax.numpy as jnp
from jax import lax
import jax.experimental.pallas as pl
import jax.experimental.pallas.tpu as pltpu

_F32 = jnp.float32
_BF16 = jnp.bfloat16
_L = 128
_EPS = 1e-5
_RING = 32


def _layernorm(x):
    m = jnp.mean(x, axis=-1, keepdims=True)
    c = x - m
    v = jnp.mean(c * c, axis=-1, keepdims=True)
    return c / jnp.sqrt(v + _EPS)


def _perm(items, k):
    m = len(items) // k
    return [items[(i % k) * m + i // k] for i in range(len(items))]


class _Stream:
    def __init__(self, sems, priority, phase):
        self.sems, self.priority, self.n = sems, priority, phase
        self.pending = {}

    def adopt(self, slot, key, src, dst):
        self.pending[slot] = (key, pltpu.make_async_copy(src, dst, self.sems.at[slot]))

    def ensure(self, key):
        for slot, (k, cp) in list(self.pending.items()):
            if k == key:
                cp.wait()
                del self.pending[slot]

    def wait_slot(self, slot):
        if slot in self.pending:
            self.pending.pop(slot)[1].wait()

    def start(self, key, src, dst):
        slot = self.n % _RING
        self.n += 1
        self.wait_slot(slot)
        cp = pltpu.make_async_copy(src, dst, self.sems.at[slot])
        cp.start(priority=self.priority)
        self.pending[slot] = (key, cp)

    def drain(self):
        for slot in list(self.pending):
            self.wait_slot(slot)


def _kernel(x_hbm, k_hbm, v_hbm, wq_hbm, wo_hbm, w3_hbm, w4_hbm, out_ref,
            xbuf, wqbuf, kbuf, vbuf, wobuf, w3buf, w4buf, qcol, slow, ssum, pb, xcol, qacc,
            sem_a, sem_b, *, H, DH, SK, W, D, F, DA, QSP, QGT, W4E, W4LS, W4P, NLX, LAG, XT, STOP, WOP, KFIRST, PACE):
    HD = H * DH
    PR = DH // 2
    NC = W // _L
    assert NC == _RING
    c0 = SK - W
    G = PR // 8
    QS, QM = wq_hbm.shape[0], wq_hbm.shape[1]
    OS, OM = wo_hbm.shape[0], wo_hbm.shape[1]

    def kv_piece(hbm, buf, row0, half, c):
        return hbm.at[pl.ds(row0, PR), pl.ds(c0 + c * _L, _L)], buf.at[half, c]

    def qk(half, c, q):
        kf = kbuf[half, c].astype(_F32)
        return jnp.sum((kf * q).reshape(G, 8, _L), axis=0)

    def pv(half, c, par, acc):
        vf = vbuf[half, c].astype(_F32)
        p = pb[par, c]
        return acc + (vf.reshape(G, 8, _L) * p[None]).reshape(PR, _L)

    def softmax_p():
        s = ssum[pl.ds(0, NC, stride=8), :]
        for r in range(1, 8):
            s = s + ssum[pl.ds(r, NC, stride=8), :]
        s = s * (DH ** -0.5)
        m = jnp.max(jnp.max(s, axis=0, keepdims=True), axis=1, keepdims=True)
        e = jnp.exp(s - m)
        l = jnp.sum(jnp.sum(e, axis=0, keepdims=True), axis=1, keepdims=True)
        return e / l

    def store_p(p, par, c):
        pb[par, c] = jnp.broadcast_to(p[c:c + 1, :], (8, _L))

    def wo_mac(osum, g, row0, att):
        oc = jnp.broadcast_to(osum[g * 8:(g + 1) * 8, :], (8, D))
        gi = row0 // 8 + g if isinstance(row0, int) else lax.shift_right_logical(row0, 3) + g
        wf = wobuf[gi // OM, gi % OM].astype(_F32) if isinstance(gi, int) else \
            wobuf[lax.shift_right_logical(gi, OM.bit_length() - 1), gi & (OM - 1)].astype(_F32)
        return att + wf * oc

    def half_slot(half, *, step, q=None, par=None, prev=None, att=None, do_softmax=None, extra=None):
        acc = jnp.zeros((PR, _L), _F32) if par is not None else None
        osum = None
        p_new = None
        for c in range(NC):
            step(c)
            if c == 0 and prev is not None:
                osum = jnp.sum(prev[0], axis=1, keepdims=True)
            if c == 0 and do_softmax is not None:
                p_new = softmax_p()
            if q is not None:
                part = qk(1 - half, c, q)
                if half == 0:
                    ssum[c * 8:(c + 1) * 8, :] = part + slow[c]
                else:
                    slow[c] = part
            if par is not None:
                acc = pv(half, c, par, acc)
            if prev is not None and 4 <= c < 4 + G:
                att = wo_mac(osum, c - 4, prev[1], att)
            if p_new is not None and 8 <= c < 24:
                store_p(p_new, do_softmax, 2 * (c - 8))
                store_p(p_new, do_softmax, 2 * (c - 8) + 1)
            if extra is not None:
                extra(c)
        return acc, att

    QW = 2 * _L
    QH = QS // 2

    def wq_piece(hf, b, c):
        sl = (pl.ds(hf * QH, QH), b, slice(None), pl.ds(c * QW, QW))
        return (("wq", hf, b, c), wq_hbm.at[sl], wqbuf.at[sl])

    bc = [(b, c) for b in range(QM) for c in range(HD // QW)]
    k_pre = [(("k", hh, c),) + kv_piece(k_hbm, kbuf, hh * PR, hh % 2, c) for hh in range(4) for c in range(NC)]
    v_pre = [(("v", 0, c),) + kv_piece(v_hbm, vbuf, 0, 0, c) for c in range(NC)]

    def wo_piece(s0, ns, b, c, w):
        sl = (pl.ds(s0, ns), b, slice(None), pl.ds(c, w))
        return (("wo",), wo_hbm.at[sl], wobuf.at[sl])

    KF = NC if KFIRST else 0
    n_kpair = len(k_pre) - 2 * KF - DA
    if WOP == "alt12":
        wo_p = [wo_piece(0, OS, b, c * _L, _L) for b in range(OM) for c in range(D // _L)]
        n_oa = (len(wo_p) - n_kpair) // 2
        wo_a = wo_p[0:2 * n_oa:2]
        wo_b = wo_p[1:2 * n_oa:2] + wo_p[2 * n_oa:]
    else:
        nb_pair = -(-n_kpair // (D // _L))
        cw = [(c, min(2 * _L, D - c)) for c in range(0, D, 2 * _L)]
        wo_a = [wo_piece(0, OS // 2, b, c, w) for b in range(OM - nb_pair) for c, w in cw]
        wo_b = ([wo_piece(OS // 2, OS // 2, b, c, w) for b in range(OM - nb_pair) for c, w in cw]
                + [wo_piece(0, OS, b, c * _L, _L) for b in range(OM - nb_pair, OM) for c in range(D // _L)])
    a_list = ([(("x",), x_hbm, xbuf)] + k_pre[:KF] + [wq_piece(0, b, c) for b, c in bc]
              + wo_a + k_pre[2 * KF:])
    b_list = k_pre[KF:2 * KF] + [wq_piece(1, b, c) for b, c in bc] + wo_b + v_pre
    T0 = len(b_list) - NC
    up_a = len(a_list) - T0
    A = _Stream(sem_a, 0, (-len(a_list)) % _RING)
    B = _Stream(sem_b, 1, (-len(b_list)) % _RING)
    for pc in a_list[:up_a]:
        A.start(*pc)
    for pc in b_list[:_RING]:
        B.start(*pc)

    A.ensure(("x",))
    x = xbuf[...].astype(_F32)
    xn = _layernorm(x).astype(_BF16).astype(_F32)

    def x_fin():
        for j in range(D // _L):
            xcol[j * _L:(j + 1) * _L, :] = jnp.broadcast_to(xn[:, j * _L:(j + 1) * _L], (_L, _L)).T

    if XT < 0:
        x_fin()

    def pre_step(t):
        B.wait_slot(B.n % _RING)
        A.start(*a_list[up_a + t])
        B.start(*b_list[t + _RING])

    def q_mac(b, c):
        A.ensure(("wq", 0, b, c))
        terms = []
        for st in range(QS):
            r = (st * QM + b) * 8
            xc = xcol[r:r + 8, :]
            terms.append(wqbuf[st, b, :, c * QW:(c + 1) * QW].astype(_F32) * jnp.concatenate([xc, xc], axis=1))
        if b > 0:
            terms.append(qacc[:, c * QW:(c + 1) * QW])
        while len(terms) > 1:
            terms = [terms[i] + terms[i + 1] if i + 1 < len(terms) else terms[i] for i in range(0, len(terms), 2)]
        qacc[:, c * QW:(c + 1) * QW] = terms[0]

    def q_fin(t0, n):
        r0 = t0 * _L if isinstance(t0, int) else pl.multiple_of(t0 * _L, _L)
        q = jnp.sum(qacc[:, pl.ds(r0, n * _L)], axis=0, keepdims=True)
        q = q.astype(_BF16).astype(_F32)
        for j in range(n):
            qcol[pl.ds(r0 + j * _L, _L), :] = jnp.broadcast_to(q[:, j * _L:(j + 1) * _L], (_L, _L)).T

    LAG = LAG + KF
    t_q = len(bc) + LAG
    t_k = T0 - 4 * NC
    QPRE = 6
    q_sched = {t_q + g * QSP: g * QGT for g in range(QPRE // QGT)}
    assert t_q < t_k + NC

    def q_extra(t):
        if t == XT:
            x_fin()
        if LAG <= t < t_q:
            q_mac(*bc[t - LAG])
        if t in q_sched:
            q_fin(q_sched[t], QGT)

    for t in range(t_k):
        if t == STOP:
            A.drain(); B.drain()
            import numpy as _np
            nb = sum(int(_np.prod(p[1].shape)) * 2 for p in a_list[:up_a + t] + b_list[:_RING + t])
            print("STOP bytes", nb, "ideal@800", nb / 800e3)
            out_ref[...] = (x + qacc[0:1, 0:1]).astype(out_ref.dtype)
            return
        pre_step(t)
        q_extra(t)

    def q_rows(row0):
        return qcol[pl.ds(row0, PR), :]

    half_slot(0, step=lambda c: pre_step(t_k + c), extra=lambda c: q_extra(t_k + c))
    half_slot(1, step=lambda c: pre_step(t_k + NC + c), q=q_rows(0), extra=lambda c: q_extra(t_k + NC + c))
    half_slot(0, step=lambda c: pre_step(t_k + 2 * NC + c), q=q_rows(PR), extra=lambda c: q_extra(t_k + 2 * NC + c))
    half_slot(1, step=lambda c: pre_step(t_k + 3 * NC + c), q=q_rows(2 * PR), do_softmax=0,
              extra=lambda c: q_extra(t_k + 3 * NC + c))
    if NLX < 0:
        A.drain(); B.drain()
        out_ref[...] = (x + qcol[0:1, 0:1] + pb[0, 0, 0:1, 0:1] + qcol[HD-1:HD, 0:1] + slow[0, 0:1, 0:1]).astype(out_ref.dtype)
        return
    A.pending.clear()
    B.pending.clear()

    def loop_step(j, half):
        r_v = pl.multiple_of(j * DH + (half + 1) * PR, 8)
        r_k = pl.multiple_of((j + 2) * DH + half * PR, 8)

        def step(c):
            pltpu.make_async_copy(*kv_piece(v_hbm, vbuf, 0, half, c), sem_b.at[c]).wait()
            pltpu.make_async_copy(*kv_piece(k_hbm, kbuf, 0, 1 - half, c), sem_a.at[c]).wait()
            pltpu.make_async_copy(*kv_piece(k_hbm, kbuf, r_k, half, c), sem_a.at[c]).start(priority=0)
            pltpu.make_async_copy(*kv_piece(v_hbm, vbuf, r_v, 1 - half, c), sem_b.at[c]).start(priority=1)
        return step

    def body(j, carry):
        acc_prev, att = carry
        par = j & 1
        r0 = pl.multiple_of(j * DH, 8)
        r_prev = pl.multiple_of(jnp.maximum(r0 - PR, 0), 8)
        acc, att = half_slot(0, step=loop_step(j, 0), q=q_rows(r0 + DH + PR), par=par,
                             prev=(acc_prev, r_prev), att=att)
        acc, att = half_slot(1, step=loop_step(j, 1), q=q_rows(r0 + 2 * DH), par=par,
                             prev=(acc, r0), att=att, do_softmax=1 - par,
                             extra=lambda c: q_fin(jnp.minimum(QPRE + 2 * j, HD // _L - 2), 2) if c == 0 else None)
        return acc, att

    NL = H - 2
    acc, att = lax.fori_loop(0, NL, body, (jnp.zeros((PR, _L), _F32), jnp.zeros((8, D), _F32)))

    A = _Stream(sem_a, 0, 0)
    B = _Stream(sem_b, 1, 0)
    for c in range(NC):
        A.adopt(c, ("k", c), *kv_piece(k_hbm, kbuf, 0, 1, c))
        B.adopt(c, ("v", c), *kv_piece(v_hbm, vbuf, 0, 0, c))
    w3_p = _perm([(("w3",), w3_hbm.at[pl.ds(r, 8), :], w3buf.at[pl.ds(r, 8), :]) for r in range(0, D, 8)], 4)

    def w4_rows(tag, r0, r1, step):
        return [((tag, r), w4_hbm.at[pl.ds(r, min(step, r1 - r)), :], w4buf.at[pl.ds(r, min(step, r1 - r)), :])
                for r in range(r0, r1, step)]

    RE = W4E * _L
    w4_e = _perm(w4_rows("w4e", 0, RE, 16), 2)
    w4_l = _perm(w4_rows("w4l", RE, F, W4LS), W4P)
    n_ma = sum(PACE)
    w4_ma = w4_l[1:2 * n_ma:2]
    w4_b = [pc for pc in w4_l if not any(pc is o for o in w4_ma)]
    assert len(w4_b) <= NC
    b_post = [(("v", hh, c),) + kv_piece(v_hbm, vbuf, hh * PR, hh % 2, c)
              for hh in range(2 * NL + 1, 2 * H) for c in range(NC)] + w4_b
    n_post = 4 * NC
    a_sched = {}
    a_early = w3_p + w4_e
    assert len(a_early) <= n_post
    for i, pc in enumerate(a_early):
        a_sched[(i * n_post) // len(a_early)] = pc

    def post_step(t):
        slot = t % _RING
        if t < len(b_post):
            B.start(*b_post[t])
        else:
            B.wait_slot(slot)
        if t < NC:
            A.ensure(("k", t))
        if t in a_sched:
            A.start(*a_sched[t])

    r30 = NL * DH
    acc, att = half_slot(0, step=lambda c: post_step(c), q=q_rows(r30 + DH + PR), par=NL & 1,
                         prev=(acc, r30 - PR), att=att)
    acc, att = half_slot(1, step=lambda c: post_step(NC + c), par=NL & 1,
                         prev=(acc, r30), att=att, do_softmax=1 - (NL & 1))
    acc, att = half_slot(0, step=lambda c: post_step(2 * NC + c), par=1 - (NL & 1),
                         prev=(acc, r30 + PR), att=att)
    acc, att = half_slot(1, step=lambda c: post_step(3 * NC + c), par=1 - (NL & 1),
                         prev=(acc, r30 + DH), att=att)

    rest_a = list(w4_ma)

    def pace(n):
        for _ in range(n):
            if rest_a:
                A.start(*rest_a.pop(0))

    osum = jnp.sum(acc, axis=1, keepdims=True)
    for g in range(G):
        att = wo_mac(osum, g, r30 + DH + PR, att)
    pace(PACE[0])
    hres = x + jnp.sum(att, axis=0, keepdims=True)
    cen = hres - jnp.mean(hres, axis=-1, keepdims=True)
    var = jnp.mean(cen * cen, axis=-1, keepdims=True)
    mc = jnp.mean(cen, axis=-1, keepdims=True)
    sd = jnp.sqrt(var + _EPS)
    x1 = cen / sd
    m2 = mc / sd
    v2 = (var - mc * mc) / (var + _EPS)
    y = jnp.broadcast_to(((x1 - m2) / jnp.sqrt(v2 + _EPS)).astype(_BF16), (8, D))
    base = hres + x1
    pace(PACE[1])
    A.ensure(("w3",))
    for pc in w4_e:
        A.ensure(pc[0])
    hid = jax.nn.gelu(jnp.dot(y, w3buf[...], preferred_element_type=_F32), approximate=True).astype(_BF16)
    base = base + jnp.dot(hid[:, :RE], w4buf[:RE, :], preferred_element_type=_F32)[0:1, :]
    hrow = hid[0:1, :].astype(_F32)
    for r in range(RE, F, _L):
        qcol[r:r + _L, :] = jnp.broadcast_to(hrow[:, r:r + _L], (_L, _L)).T
    tail = None
    for (_, r), _, _ in w4_l:
        A.ensure(("w4l", r))
        B.ensure(("w4l", r))
        for rr in range(r, r + W4LS, 8):
            hc = qcol[rr:rr + 8, :]
            term = w4buf[rr:rr + 8, :].astype(_F32) * jnp.concatenate([hc] * (D // _L), axis=1)
            tail = term if tail is None else tail + term
    A.drain()
    B.drain()
    out_ref[...] = (base + jnp.sum(tail, axis=0, keepdims=True)).astype(out_ref.dtype)


def _build(A_x, A_k_cache, A_v_cache, A_wq, A_wo, B_w3, B_w4, *, DA=12, QSP=13, QGT=2, W4E=4, W4LS=32, W4P=2, NLX=0, LAG=8, XT=-1, STOP=-1, WOP='half6', KFIRST=True, PACE=(2, 3)):
    B, S, D = A_x.shape
    _, H, SK, DH = A_k_cache.shape
    assert B == 1 and S == 1
    W = min(4096, max(256, SK // 4))
    F = B_w3.shape[1]
    HD = H * DH
    PR = DH // 2
    NC = W // _L
    kt = jnp.swapaxes(A_k_cache[0], 1, 2).reshape(HD, SK)
    vt = jnp.swapaxes(A_v_cache[0], 1, 2).reshape(HD, SK)
    x2 = A_x.reshape(1, D)
    wq4 = A_wq.reshape(10, D // 80, 8, HD)
    wo4 = A_wo.reshape(12, HD // 96, 8, D)
    kern = functools.partial(_kernel, H=H, DH=DH, SK=SK, W=W, D=D, F=F, DA=DA, QSP=QSP, QGT=QGT, W4E=W4E, W4LS=W4LS, W4P=W4P, NLX=NLX, LAG=LAG, XT=XT, STOP=STOP, WOP=WOP, KFIRST=KFIRST, PACE=PACE)
    dma = pltpu.SemaphoreType.DMA
    out = pl.pallas_call(
        kern,
        out_shape=jax.ShapeDtypeStruct((1, D), A_x.dtype),
        in_specs=[pl.BlockSpec(memory_space=pl.ANY)] * 7,
        out_specs=pl.BlockSpec(memory_space=pltpu.VMEM),
        scratch_shapes=[
            pltpu.VMEM((1, D), A_x.dtype),
            pltpu.VMEM(wq4.shape, A_wq.dtype),
            pltpu.VMEM((2, NC, PR, _L), A_k_cache.dtype),
            pltpu.VMEM((2, NC, PR, _L), A_v_cache.dtype),
            pltpu.VMEM(wo4.shape, A_wo.dtype),
            pltpu.VMEM((D, F), B_w3.dtype),
            pltpu.VMEM((F, D), B_w4.dtype),
            pltpu.VMEM((HD, _L), _F32),
            pltpu.VMEM((NC, 8, _L), _F32),
            pltpu.VMEM((NC * 8, _L), _F32),
            pltpu.VMEM((2, NC, 8, _L), _F32),
            pltpu.VMEM((D, _L), _F32),
            pltpu.VMEM((8, HD), _F32),
            dma((_RING,)), dma((_RING,)),
        ],
        compiler_params=pltpu.CompilerParams(
            vmem_limit_bytes=64 * 1024 * 1024,
            disable_bounds_checks=True,
            disable_semaphore_checks=True,
        ),
    )(x2, kt, vt, wq4, wo4, B_w3, B_w4)
    return out.reshape(B, S, D)


@jax.jit
def pallas_sequential_preLN__sliding_block_cached__mixer_s_mlp__decode_kernel(
    A_x: jax.Array,
    A_k_cache: jax.Array,
    A_v_cache: jax.Array,
    A_wq: jax.Array,
    A_wo: jax.Array,
    B_x: jax.Array,
    B_w1: jax.Array,
    B_w2: jax.Array,
    B_w3: jax.Array,
    B_w4: jax.Array,
):
    return _build(A_x, A_k_cache, A_v_cache, A_wq, A_wo, B_w3, B_w4)
```

```python
import functools

import jax
import jax.numpy as jnp
from jax import lax
import jax.experimental.pallas as pl
import jax.experimental.pallas.tpu as pltpu

_F32 = jnp.float32
_BF16 = jnp.bfloat16
_L = 128
_EPS = 1e-5
_RING = 32


def _layernorm(x):
    m = jnp.mean(x, axis=-1, keepdims=True)
    c = x - m
    v = jnp.mean(c * c, axis=-1, keepdims=True)
    return c / jnp.sqrt(v + _EPS)


def _columns(row):
    return jnp.broadcast_to(row, (_L, _L)).T


def _perm(items, k):
    m = len(items) // k
    assert m * k == len(items)
    return [items[(i % k) * m + i // k] for i in range(len(items))]


class _Stream:
    def __init__(self, sems, priority, phase):
        self.sems, self.priority, self.n = sems, priority, phase
        self.pending = {}

    def adopt(self, slot, key, src, dst):
        self.pending[slot] = (key, pltpu.make_async_copy(src, dst, self.sems.at[slot]))

    def ensure(self, key):
        for slot, (k, _) in list(self.pending.items()):
            if k == key:
                self.wait_slot(slot)

    def wait_slot(self, slot):
        if slot in self.pending:
            self.pending.pop(slot)[1].wait()

    def start(self, key, src, dst):
        slot = self.n % _RING
        self.n += 1
        self.wait_slot(slot)
        cp = pltpu.make_async_copy(src, dst, self.sems.at[slot])
        cp.start(priority=self.priority)
        self.pending[slot] = (key, cp)

    def drain(self):
        for slot in list(self.pending):
            self.wait_slot(slot)


def _kernel(x_hbm, k_hbm, v_hbm, wq_hbm, wo_hbm, w3_hbm, w4_hbm, out_ref,
            xbuf, wqbuf, kbuf, vbuf, wobuf, w3buf, w4buf, qcol, slow, ssum, pb, xcol, qacc,
            sem_a, sem_b, *, H, DH, W, DA, LAG, W4E, W4LS, PACE):
    HD, SK = k_hbm.shape
    D, F = w3_hbm.shape
    PR = DH // 2
    NC = W // _L
    G = PR // 8
    DT = D // _L
    WS, WM = wq_hbm.shape[:2]
    assert NC == _RING and WM & (WM - 1) == 0 and wo_hbm.shape == wq_hbm.shape

    def kv_piece(hbm, buf, row0, half, c):
        return hbm.at[pl.ds(row0, PR), pl.ds(SK - W + c * _L, _L)], buf.at[half, c]

    def q_rows(row0):
        return qcol[pl.ds(row0, PR), :]

    def softmax_p():
        s = ssum[pl.ds(0, NC, stride=8), :]
        for r in range(1, 8):
            s = s + ssum[pl.ds(r, NC, stride=8), :]
        s = s * (DH ** -0.5)
        m = jnp.max(jnp.max(s, axis=0, keepdims=True), axis=1, keepdims=True)
        e = jnp.exp(s - m)
        return e / jnp.sum(jnp.sum(e, axis=0, keepdims=True), axis=1, keepdims=True)

    def wo_mac(o, g, row0, att):
        if isinstance(row0, int):
            tiles = [wobuf[divmod((row0 // 8 + g) * DT + n, WM)] for n in range(DT)]
        else:
            t = (lax.shift_right_logical(row0, 3) + g) * DT
            tiles = [wobuf[lax.shift_right_logical(t + n, WM.bit_length() - 1), (t + n) & (WM - 1)]
                     for n in range(DT)]
        w = jnp.concatenate([tl.astype(_F32) for tl in tiles], axis=1)
        return att + w * jnp.broadcast_to(o[g * 8:(g + 1) * 8, :], (8, D))

    def half_slot(half, step, *, q=None, kslot=None, par=None, prev=None, att=None, p_out=None, extra=None):
        acc = None if par is None else jnp.zeros((PR, _L), _F32)
        o = p_new = None
        for c in range(NC):
            step(c)
            if c == 0 and prev is not None:
                o = jnp.sum(prev[0], axis=1, keepdims=True)
            if c == 0 and p_out is not None:
                p_new = softmax_p()
            if q is not None:
                part = jnp.sum((kbuf[1 - half if kslot is None else kslot, c].astype(_F32) * q).reshape(G, 8, _L), axis=0)
                if half == 0:
                    ssum[c * 8:(c + 1) * 8, :] = part + slow[c]
                else:
                    slow[c] = part
            if par is not None:
                vf = vbuf[half, c].astype(_F32).reshape(G, 8, _L)
                acc = acc + (vf * pb[par, c][None]).reshape(PR, _L)
            if prev is not None and 4 <= c < 4 + G:
                att = wo_mac(o, c - 4, prev[1], att)
            if p_out is not None and 8 <= c < 8 + NC // 2:
                for i in (2 * (c - 8), 2 * (c - 8) + 1):
                    pb[p_out, i] = jnp.broadcast_to(p_new[i:i + 1, :], (8, _L))
            if extra is not None:
                extra(c)
        return acc, att

    QW = 2 * _L

    def w_piece(key, hbm, buf, t, s0=0, s1=WS):
        return key, hbm.at[s0:s1, t], buf.at[s0:s1, t]

    k_p = [[(None,) + kv_piece(k_hbm, kbuf, hh * PR, sl, c) for c in range(NC)]
           for hh, sl in enumerate((2, 1, 0, 1))]
    v_p = [(None,) + kv_piece(v_hbm, vbuf, 0, 0, c) for c in range(NC)]
    n0 = LAG + 2
    n1 = WM - 3 * NC - n0
    n2 = WM - (NC - DA)
    SH = WS // 2
    a_list = ([("x", x_hbm, xbuf)]
              + [w_piece(("wq", t), wq_hbm, wqbuf, t, 0, SH if t < n0 else WS) for t in range(WM)]
              + [w_piece(None, wo_hbm, wobuf, t, 0, SH) for t in range(n1, n2)] + k_p[3])
    b_list = ([w_piece(None, wq_hbm, wqbuf, t, SH, WS) for t in range(n0)] + k_p[0] + k_p[1] + k_p[2]
              + [w_piece(None, wo_hbm, wobuf, t, SH if n1 <= t < n2 else 0, WS) for t in range(WM)] + v_p)
    T0 = len(b_list) - NC
    up_a = len(a_list) - T0
    A = _Stream(sem_a, 0, -len(a_list) % _RING)
    B = _Stream(sem_b, 1, -len(b_list) % _RING)
    for pc in a_list[:up_a]:
        A.start(*pc)
    for pc in b_list[:_RING]:
        B.start(*pc)

    A.ensure("x")
    x = xbuf[...].astype(_F32)
    xn = _layernorm(x).astype(_BF16).astype(_F32)
    for j in range(0, D, _L):
        xcol[j:j + _L, :] = _columns(xn[:, j:j + _L])

    touched = set()

    def q_mac(t):
        A.ensure(("wq", t))
        terms = {}
        for st in range(WS):
            rt, ct = divmod(st * WM + t, HD // _L)
            terms.setdefault(ct, []).append(wqbuf[st, t].astype(_F32) * xcol[rt * 8:(rt + 1) * 8, :])
        for ct, ts in terms.items():
            if ct in touched:
                ts.append(qacc[:, ct * _L:(ct + 1) * _L])
            touched.add(ct)
            while len(ts) > 1:
                ts = [sum(ts[i + 1:i + 2], ts[i]) for i in range(0, len(ts), 2)]
            qacc[:, ct * _L:(ct + 1) * _L] = ts[0]

    def q_fin(r0):
        q = jnp.sum(qacc[:, pl.ds(r0, QW)], axis=0, keepdims=True).astype(_BF16).astype(_F32)
        for j in range(0, QW, _L):
            qcol[pl.ds(r0 + j, _L), :] = _columns(q[:, j:j + _L])

    t_q = LAG + WM
    t_k = T0 - 3 * NC
    NQP = 3
    assert t_q < t_k

    def pre_step(t):
        B.wait_slot(B.n % _RING)
        A.start(*a_list[up_a + t])
        B.start(*b_list[t + _RING])

    for t in range(t_k):
        pre_step(t)
        if LAG <= t < t_q:
            q_mac(t - LAG)
        if t == t_q:
            q_fin(0)
    half_slot(1, lambda c: pre_step(t_k + c), q=q_rows(0), kslot=2)
    half_slot(0, lambda c: pre_step(t_k + NC + c), q=q_rows(PR), extra=lambda c: q_fin(QW) if c == 0 else None)
    half_slot(1, lambda c: pre_step(t_k + 2 * NC + c), q=q_rows(DH), p_out=0,
              extra=lambda c: q_fin(2 * QW) if c == 0 else None)

    def loop_step(j, half):
        r_k = pl.multiple_of((j + 2) * DH + half * PR, 8)
        r_v = pl.multiple_of(j * DH + (half + 1) * PR, 8)

        def step(c):
            pltpu.make_async_copy(*kv_piece(v_hbm, vbuf, 0, half, c), sem_b.at[c]).wait()
            pltpu.make_async_copy(*kv_piece(k_hbm, kbuf, 0, 1 - half, c), sem_a.at[c]).wait()
            pltpu.make_async_copy(*kv_piece(k_hbm, kbuf, r_k, half, c), sem_a.at[c]).start(priority=0)
            pltpu.make_async_copy(*kv_piece(v_hbm, vbuf, r_v, 1 - half, c), sem_b.at[c]).start(priority=1)
        return step

    def head(j, carry):
        acc, att = carry
        par = j & 1
        r0 = pl.multiple_of(j * DH, 8)
        r_q = pl.multiple_of(jnp.minimum((NQP + j) * QW, HD - QW), _L)
        acc, att = half_slot(0, loop_step(j, 0), q=q_rows(r0 + DH + PR), par=par,
                             prev=(acc, jnp.maximum(r0 - PR, 0)), att=att)
        return half_slot(1, loop_step(j, 1), q=q_rows(r0 + 2 * DH), par=par, prev=(acc, r0), att=att,
                         p_out=1 - par, extra=lambda c: q_fin(r_q) if c == 0 else None)

    NL = H - 2
    acc, att = lax.fori_loop(0, NL, head, (jnp.zeros((PR, _L), _F32), jnp.zeros((8, D), _F32)))

    A = _Stream(sem_a, 0, 0)
    B = _Stream(sem_b, 1, 0)
    for c in range(NC):
        A.adopt(c, ("k", c), *kv_piece(k_hbm, kbuf, 0, 1, c))
        B.adopt(c, None, *kv_piece(v_hbm, vbuf, 0, 0, c))

    def rows(key, hbm, buf, r0, r1, n):
        return [(key or r, hbm.at[pl.ds(r, n), :], buf.at[pl.ds(r, n), :]) for r in range(r0, r1, n)]

    RE = W4E * _L
    a_early = _perm(rows("w", w3_hbm, w3buf, 0, D, 8), 4) + _perm(rows("w", w4_hbm, w4buf, 0, RE, 16), 2)
    w4_late = _perm(rows(None, w4_hbm, w4buf, RE, F, W4LS), 2)
    late_a = w4_late[1:2 * sum(PACE):2]
    b_post = ([(None,) + kv_piece(v_hbm, vbuf, hh * PR, hh % 2, c)
               for hh in range(2 * NL + 1, 2 * H) for c in range(NC)]
              + [pc for pc in w4_late if not any(pc is o for o in late_a)])
    assert len(b_post) <= 4 * NC and len(a_early) <= 4 * NC
    a_sched = {(i * 4 * NC) // len(a_early): pc for i, pc in enumerate(a_early)}

    def post_step(t):
        B.wait_slot(t % _RING)
        A.ensure(("k", t))
        if t in a_sched:
            A.start(*a_sched[t])
        if t < len(b_post):
            B.start(*b_post[t])

    r0, par = NL * DH, NL & 1
    acc, att = half_slot(0, post_step, q=q_rows(r0 + DH + PR), par=par, prev=(acc, r0 - PR), att=att)
    acc, att = half_slot(1, lambda c: post_step(NC + c), par=par, prev=(acc, r0), att=att, p_out=1 - par)
    acc, att = half_slot(0, lambda c: post_step(2 * NC + c), par=1 - par, prev=(acc, r0 + PR), att=att)
    acc, att = half_slot(1, lambda c: post_step(3 * NC + c), par=1 - par, prev=(acc, r0 + DH), att=att)

    o = jnp.sum(acc, axis=1, keepdims=True)
    for g in range(G):
        att = wo_mac(o, g, r0 + DH + PR, att)
    for pc in late_a[:PACE[0]]:
        A.start(*pc)
    hres = x + jnp.sum(att, axis=0, keepdims=True)
    x1 = _layernorm(hres)
    y = jnp.broadcast_to(_layernorm(x1).astype(_BF16), (8, D))
    for pc in late_a[PACE[0]:]:
        A.start(*pc)
    A.ensure("w")
    hid = jax.nn.gelu(jnp.dot(y, w3buf[...], preferred_element_type=_F32), approximate=True).astype(_BF16)
    res = hres + x1 + jnp.dot(hid[:, :RE], w4buf[:RE, :], preferred_element_type=_F32)[0:1, :]
    hrow = hid[0:1, :].astype(_F32)
    for r in range(RE, F, _L):
        qcol[r:r + _L, :] = _columns(hrow[:, r:r + _L])
    tail = jnp.zeros((8, D), _F32)
    for r, _, _ in w4_late:
        A.ensure(r)
        B.ensure(r)
        for rr in range(r, r + W4LS, 8):
            hc = jnp.concatenate([qcol[rr:rr + 8, :]] * (D // _L), axis=1)
            tail = tail + w4buf[rr:rr + 8, :].astype(_F32) * hc
    A.drain()
    B.drain()
    out_ref[...] = (res + jnp.sum(tail, axis=0, keepdims=True)).astype(out_ref.dtype)


def _tile_streams(w):
    r, c = w.shape
    return w.reshape(r // 8, 8, c // _L, _L).transpose(0, 2, 1, 3).reshape(-1, 256, 8, _L)


def _compiler_params():
    base = dict(vmem_limit_bytes=48 * 1024 * 1024)
    try:
        return pltpu.CompilerParams(disable_bounds_checks=True, disable_semaphore_checks=True, **base)
    except TypeError:
        return pltpu.CompilerParams(**base)


def _build(A_x, A_k_cache, A_v_cache, A_wq, A_wo, B_w3, B_w4, *, DA=12, LAG=6, W4E=4, W4LS=32, PACE=(3, 4)):
    B, S, D = A_x.shape
    _, H, SK, DH = A_k_cache.shape
    assert B == 1 and S == 1
    W = min(4096, max(256, SK // 4))
    HD = H * DH
    NC = W // _L
    kt = jnp.swapaxes(A_k_cache[0], 1, 2).reshape(HD, SK)
    vt = jnp.swapaxes(A_v_cache[0], 1, 2).reshape(HD, SK)
    wq4 = _tile_streams(A_wq)
    wo4 = _tile_streams(A_wo)
    out = pl.pallas_call(
        functools.partial(_kernel, H=H, DH=DH, W=W, DA=DA, LAG=LAG, W4E=W4E, W4LS=W4LS, PACE=PACE),
        out_shape=jax.ShapeDtypeStruct((1, D), A_x.dtype),
        in_specs=[pl.BlockSpec(memory_space=pl.ANY)] * 7,
        out_specs=pl.BlockSpec(memory_space=pltpu.VMEM),
        scratch_shapes=[
            pltpu.VMEM((1, D), A_x.dtype),
            pltpu.VMEM(wq4.shape, A_wq.dtype),
            pltpu.VMEM((3, NC, DH // 2, _L), A_k_cache.dtype),
            pltpu.VMEM((2, NC, DH // 2, _L), A_v_cache.dtype),
            pltpu.VMEM(wo4.shape, A_wo.dtype),
            pltpu.VMEM(B_w3.shape, B_w3.dtype),
            pltpu.VMEM(B_w4.shape, B_w4.dtype),
            pltpu.VMEM((HD, _L), _F32),
            pltpu.VMEM((NC, 8, _L), _F32),
            pltpu.VMEM((NC * 8, _L), _F32),
            pltpu.VMEM((2, NC, 8, _L), _F32),
            pltpu.VMEM((D, _L), _F32),
            pltpu.VMEM((8, HD), _F32),
            pltpu.SemaphoreType.DMA((_RING,)),
            pltpu.SemaphoreType.DMA((_RING,)),
        ],
        compiler_params=_compiler_params(),
    )(A_x.reshape(1, D), kt, vt, wq4, wo4, B_w3, B_w4)
    return out.reshape(B, S, D)


@jax.jit
def pallas_sequential_preLN__sliding_block_cached__mixer_s_mlp__decode_kernel(
    A_x: jax.Array,
    A_k_cache: jax.Array,
    A_v_cache: jax.Array,
    A_wq: jax.Array,
    A_wo: jax.Array,
    B_x: jax.Array,
    B_w1: jax.Array,
    B_w2: jax.Array,
    B_w3: jax.Array,
    B_w4: jax.Array,
):
    return _build(A_x, A_k_cache, A_v_cache, A_wq, A_wo, B_w3, B_w4)
```

```python
import functools

import jax
import jax.numpy as jnp
from jax import lax
import jax.experimental.pallas as pl
import jax.experimental.pallas.tpu as pltpu

_F32 = jnp.float32
_BF16 = jnp.bfloat16
_L = 128
_EPS = 1e-5
_RING = 32


def _layernorm(x):
    m = jnp.mean(x, axis=-1, keepdims=True)
    c = x - m
    v = jnp.mean(c * c, axis=-1, keepdims=True)
    return c / jnp.sqrt(v + _EPS)


def _columns(row):
    return jnp.broadcast_to(row, (_L, _L)).T


def _perm(items, k):
    m = len(items) // k
    assert m * k == len(items)
    return [items[(i % k) * m + i // k] for i in range(len(items))]


class _Stream:
    def __init__(self, sems, priority, phase):
        self.sems, self.priority, self.n = sems, priority, phase
        self.pending = {}

    def adopt(self, slot, key, src, dst):
        self.pending[slot] = (key, pltpu.make_async_copy(src, dst, self.sems.at[slot]))

    def ensure(self, key):
        for slot, (k, _) in list(self.pending.items()):
            if k == key:
                self.wait_slot(slot)

    def wait_slot(self, slot):
        if slot in self.pending:
            self.pending.pop(slot)[1].wait()

    def start(self, key, src, dst):
        slot = self.n % _RING
        self.n += 1
        self.wait_slot(slot)
        cp = pltpu.make_async_copy(src, dst, self.sems.at[slot])
        cp.start(priority=self.priority)
        self.pending[slot] = (key, cp)

    def drain(self):
        for slot in list(self.pending):
            self.wait_slot(slot)


def _kernel(x_hbm, k_hbm, v_hbm, wq_hbm, wo_hbm, w3_hbm, w4_hbm, out_ref,
            xbuf, wqbuf, kbuf, vbuf, wobuf, w3buf, w4buf, qcol, slow, ssum, pb, xcol, qacc,
            sem_a, sem_b, *, H, DH, W, DA, W4E, W4LS, PACE):
    HD, SK = k_hbm.shape
    D, F = w3_hbm.shape
    PR = DH // 2
    NC = W // _L
    G = PR // 8
    DT = D // _L
    WS, WM = wq_hbm.shape[:2]
    assert NC == _RING and WM & (WM - 1) == 0 and wo_hbm.shape == wq_hbm.shape

    def kv_piece(hbm, buf, row0, half, c):
        return hbm.at[pl.ds(row0, PR), pl.ds(SK - W + c * _L, _L)], buf.at[half, c]

    def q_rows(row0):
        return qcol[pl.ds(row0, PR), :]

    def softmax_p():
        s = ssum[pl.ds(0, NC, stride=8), :]
        for r in range(1, 8):
            s = s + ssum[pl.ds(r, NC, stride=8), :]
        s = s * (DH ** -0.5)
        m = jnp.max(jnp.max(s, axis=0, keepdims=True), axis=1, keepdims=True)
        e = jnp.exp(s - m)
        return e / jnp.sum(jnp.sum(e, axis=0, keepdims=True), axis=1, keepdims=True)

    def wo_mac(o, g, row0, att):
        if isinstance(row0, int):
            tiles = [wobuf[divmod((row0 // 8 + g) * DT + n, WM)] for n in range(DT)]
        else:
            t = (lax.shift_right_logical(row0, 3) + g) * DT
            tiles = [wobuf[lax.shift_right_logical(t + n, WM.bit_length() - 1), (t + n) & (WM - 1)]
                     for n in range(DT)]
        w = jnp.concatenate([tl.astype(_F32) for tl in tiles], axis=1)
        return att + w * jnp.broadcast_to(o[g * 8:(g + 1) * 8, :], (8, D))

    def half_slot(half, step, *, q=None, kslot=None, par=None, prev=None, att=None, p_out=None, extra=None):
        acc = None if par is None else jnp.zeros((PR, _L), _F32)
        o = p_new = None
        for c in range(NC):
            step(c)
            if c == 0 and prev is not None:
                o = jnp.sum(prev[0], axis=1, keepdims=True)
            if c == 0 and p_out is not None:
                p_new = softmax_p()
            if q is not None:
                part = jnp.sum((kbuf[1 - half if kslot is None else kslot, c].astype(_F32) * q).reshape(G, 8, _L), axis=0)
                if half == 0:
                    ssum[c * 8:(c + 1) * 8, :] = part + slow[c]
                else:
                    slow[c] = part
            if par is not None:
                vf = vbuf[half, c].astype(_F32).reshape(G, 8, _L)
                acc = acc + (vf * pb[par, c][None]).reshape(PR, _L)
            if prev is not None and 4 <= c < 4 + G:
                att = wo_mac(o, c - 4, prev[1], att)
            if p_out is not None and 8 <= c < 8 + NC // 2:
                for i in (2 * (c - 8), 2 * (c - 8) + 1):
                    pb[p_out, i] = jnp.broadcast_to(p_new[i:i + 1, :], (8, _L))
            if extra is not None:
                extra(c)
        return acc, att

    QW = 2 * _L

    def w_piece(key, hbm, buf, t, s0=0, s1=WS):
        return key, hbm.at[s0:s1, t], buf.at[s0:s1, t]

    k_p = [[(None,) + kv_piece(k_hbm, kbuf, hh * PR, sl, c) for c in range(NC)]
           for hh, sl in enumerate((2, 1, 0, 1))]
    v_p = [(None,) + kv_piece(v_hbm, vbuf, 0, 0, c) for c in range(NC)]
    n1 = WM - 3 * NC
    n2 = WM - (NC - DA)
    SH = WS // 2
    a_list = ([("x", x_hbm, xbuf)] + k_p[0] + k_p[1] + k_p[2]
              + [w_piece(None, wo_hbm, wobuf, t, 0, WS if t < n1 else SH) for t in range(n2)] + k_p[3])
    b_list = ([w_piece(None, wq_hbm, wqbuf, t) for t in range(WM)]
              + [w_piece(None, wo_hbm, wobuf, t, SH if t < n2 else 0, WS) for t in range(n1, WM)] + v_p)
    T0 = len(b_list) - NC
    up_a = len(a_list) - T0
    A = _Stream(sem_a, 0, -len(a_list) % _RING)
    B = _Stream(sem_b, 1, -len(b_list) % _RING)
    for pc in a_list[:up_a]:
        A.start(*pc)
    for pc in b_list[:_RING]:
        B.start(*pc)

    A.ensure("x")
    x = xbuf[...].astype(_F32)
    xn = _layernorm(x).astype(_BF16).astype(_F32)
    for j in range(0, D, _L):
        xcol[j:j + _L, :] = _columns(xn[:, j:j + _L])

    touched = set()

    def q_mac(t):
        terms = {}
        for st in range(WS):
            rt, ct = divmod(st * WM + t, HD // _L)
            terms.setdefault(ct, []).append(wqbuf[st, t].astype(_F32) * xcol[rt * 8:(rt + 1) * 8, :])
        for ct, ts in terms.items():
            if ct in touched:
                ts.append(qacc[:, ct * _L:(ct + 1) * _L])
            touched.add(ct)
            while len(ts) > 1:
                ts = [sum(ts[i + 1:i + 2], ts[i]) for i in range(0, len(ts), 2)]
            qacc[:, ct * _L:(ct + 1) * _L] = ts[0]

    def q_fin(r0):
        q = jnp.sum(qacc[:, pl.ds(r0, QW)], axis=0, keepdims=True).astype(_BF16).astype(_F32)
        for j in range(0, QW, _L):
            qcol[pl.ds(r0 + j, _L), :] = _columns(q[:, j:j + _L])

    t_k = T0 - 3 * NC
    NQP = 3
    assert t_k == WM

    def pre_step(t):
        B.wait_slot(B.n % _RING)
        A.start(*a_list[up_a + t])
        B.start(*b_list[t + _RING])

    for t in range(t_k):
        pre_step(t)
        q_mac(t)
    q_fin(0)
    half_slot(1, lambda c: pre_step(t_k + c), q=q_rows(0), kslot=2)
    half_slot(0, lambda c: pre_step(t_k + NC + c), q=q_rows(PR), extra=lambda c: q_fin(QW) if c == 0 else None)
    half_slot(1, lambda c: pre_step(t_k + 2 * NC + c), q=q_rows(DH), p_out=0,
              extra=lambda c: q_fin(2 * QW) if c == 0 else None)

    def loop_step(j, half):
        r_k = pl.multiple_of((j + 2) * DH + half * PR, 8)
        r_v = pl.multiple_of(j * DH + (half + 1) * PR, 8)

        def step(c):
            pltpu.make_async_copy(*kv_piece(v_hbm, vbuf, 0, half, c), sem_b.at[c]).wait()
            pltpu.make_async_copy(*kv_piece(k_hbm, kbuf, 0, 1 - half, c), sem_a.at[c]).wait()
            pltpu.make_async_copy(*kv_piece(k_hbm, kbuf, r_k, half, c), sem_a.at[c]).start(priority=0)
            pltpu.make_async_copy(*kv_piece(v_hbm, vbuf, r_v, 1 - half, c), sem_b.at[c]).start(priority=1)
        return step

    def head(j, carry):
        acc, att = carry
        par = j & 1
        r0 = pl.multiple_of(j * DH, 8)
        r_q = pl.multiple_of(jnp.minimum((NQP + j) * QW, HD - QW), _L)
        acc, att = half_slot(0, loop_step(j, 0), q=q_rows(r0 + DH + PR), par=par,
                             prev=(acc, jnp.maximum(r0 - PR, 0)), att=att)
        return half_slot(1, loop_step(j, 1), q=q_rows(r0 + 2 * DH), par=par, prev=(acc, r0), att=att,
                         p_out=1 - par, extra=lambda c: q_fin(r_q) if c == 0 else None)

    NL = H - 2
    acc, att = lax.fori_loop(0, NL, head, (jnp.zeros((PR, _L), _F32), jnp.zeros((8, D), _F32)))

    A = _Stream(sem_a, 0, 0)
    B = _Stream(sem_b, 1, 0)
    for c in range(NC):
        A.adopt(c, ("k", c), *kv_piece(k_hbm, kbuf, 0, 1, c))
        B.adopt(c, None, *kv_piece(v_hbm, vbuf, 0, 0, c))

    def rows(key, hbm, buf, r0, r1, n):
        return [(key or r, hbm.at[pl.ds(r, n), :], buf.at[pl.ds(r, n), :]) for r in range(r0, r1, n)]

    RE = W4E * _L
    a_early = _perm(rows("w", w3_hbm, w3buf, 0, D, 8), 4) + _perm(rows("w", w4_hbm, w4buf, 0, RE, 16), 2)
    w4_late = _perm(rows(None, w4_hbm, w4buf, RE, F, W4LS), 2)
    late_a = w4_late[1:2 * sum(PACE):2]
    b_post = ([(None,) + kv_piece(v_hbm, vbuf, hh * PR, hh % 2, c)
               for hh in range(2 * NL + 1, 2 * H) for c in range(NC)]
              + [pc for pc in w4_late if not any(pc is o for o in late_a)])
    assert len(b_post) <= 4 * NC and len(a_early) <= 4 * NC
    a_sched = {(i * 4 * NC) // len(a_early): pc for i, pc in enumerate(a_early)}

    def post_step(t):
        B.wait_slot(t % _RING)
        A.ensure(("k", t))
        if t in a_sched:
            A.start(*a_sched[t])
        if t < len(b_post):
            B.start(*b_post[t])

    r0, par = NL * DH, NL & 1
    acc, att = half_slot(0, post_step, q=q_rows(r0 + DH + PR), par=par, prev=(acc, r0 - PR), att=att)
    acc, att = half_slot(1, lambda c: post_step(NC + c), par=par, prev=(acc, r0), att=att, p_out=1 - par)
    acc, att = half_slot(0, lambda c: post_step(2 * NC + c), par=1 - par, prev=(acc, r0 + PR), att=att)
    acc, att = half_slot(1, lambda c: post_step(3 * NC + c), par=1 - par, prev=(acc, r0 + DH), att=att)

    o = jnp.sum(acc, axis=1, keepdims=True)
    for g in range(G):
        att = wo_mac(o, g, r0 + DH + PR, att)
    for pc in late_a[:PACE[0]]:
        A.start(*pc)
    hres = x + jnp.sum(att, axis=0, keepdims=True)
    x1 = _layernorm(hres)
    y = jnp.broadcast_to(_layernorm(x1).astype(_BF16), (8, D))
    for pc in late_a[PACE[0]:]:
        A.start(*pc)
    A.ensure("w")
    hid = jax.nn.gelu(jnp.dot(y, w3buf[...], preferred_element_type=_F32), approximate=True).astype(_BF16)
    res = hres + x1 + jnp.dot(hid[:, :RE], w4buf[:RE, :], preferred_element_type=_F32)[0:1, :]
    hrow = hid[0:1, :].astype(_F32)
    for r in range(RE, F, _L):
        qcol[r:r + _L, :] = _columns(hrow[:, r:r + _L])
    tail = jnp.zeros((8, D), _F32)
    for r, _, _ in w4_late:
        A.ensure(r)
        B.ensure(r)
        for rr in range(r, r + W4LS, 8):
            hc = jnp.concatenate([qcol[rr:rr + 8, :]] * (D // _L), axis=1)
            tail = tail + w4buf[rr:rr + 8, :].astype(_F32) * hc
    A.drain()
    B.drain()
    out_ref[...] = (res + jnp.sum(tail, axis=0, keepdims=True)).astype(out_ref.dtype)


def _tile_streams(w):
    r, c = w.shape
    return w.reshape(r // 8, 8, c // _L, _L).transpose(0, 2, 1, 3).reshape(-1, 256, 8, _L)


def _compiler_params():
    base = dict(vmem_limit_bytes=48 * 1024 * 1024)
    try:
        return pltpu.CompilerParams(disable_bounds_checks=True, disable_semaphore_checks=True, **base)
    except TypeError:
        return pltpu.CompilerParams(**base)


def _build(A_x, A_k_cache, A_v_cache, A_wq, A_wo, B_w3, B_w4, *, DA=12, W4E=4, W4LS=32, PACE=(3, 4)):
    B, S, D = A_x.shape
    _, H, SK, DH = A_k_cache.shape
    assert B == 1 and S == 1
    W = min(4096, max(256, SK // 4))
    HD = H * DH
    NC = W // _L
    kt = jnp.swapaxes(A_k_cache[0], 1, 2).reshape(HD, SK)
    vt = jnp.swapaxes(A_v_cache[0], 1, 2).reshape(HD, SK)
    wq4 = _tile_streams(A_wq)
    wo4 = _tile_streams(A_wo)
    out = pl.pallas_call(
        functools.partial(_kernel, H=H, DH=DH, W=W, DA=DA, W4E=W4E, W4LS=W4LS, PACE=PACE),
        out_shape=jax.ShapeDtypeStruct((1, D), A_x.dtype),
        in_specs=[pl.BlockSpec(memory_space=pl.ANY)] * 7,
        out_specs=pl.BlockSpec(memory_space=pltpu.VMEM),
        scratch_shapes=[
            pltpu.VMEM((1, D), A_x.dtype),
            pltpu.VMEM(wq4.shape, A_wq.dtype),
            pltpu.VMEM((3, NC, DH // 2, _L), A_k_cache.dtype),
            pltpu.VMEM((2, NC, DH // 2, _L), A_v_cache.dtype),
            pltpu.VMEM(wo4.shape, A_wo.dtype),
            pltpu.VMEM(B_w3.shape, B_w3.dtype),
            pltpu.VMEM(B_w4.shape, B_w4.dtype),
            pltpu.VMEM((HD, _L), _F32),
            pltpu.VMEM((NC, 8, _L), _F32),
            pltpu.VMEM((NC * 8, _L), _F32),
            pltpu.VMEM((2, NC, 8, _L), _F32),
            pltpu.VMEM((D, _L), _F32),
            pltpu.VMEM((8, HD), _F32),
            pltpu.SemaphoreType.DMA((_RING,)),
            pltpu.SemaphoreType.DMA((_RING,)),
        ],
        compiler_params=_compiler_params(),
    )(A_x.reshape(1, D), kt, vt, wq4, wo4, B_w3, B_w4)
    return out.reshape(B, S, D)


@jax.jit
def pallas_sequential_preLN__sliding_block_cached__mixer_s_mlp__decode_kernel(
    A_x: jax.Array,
    A_k_cache: jax.Array,
    A_v_cache: jax.Array,
    A_wq: jax.Array,
    A_wo: jax.Array,
    B_x: jax.Array,
    B_w1: jax.Array,
    B_w2: jax.Array,
    B_w3: jax.Array,
    B_w4: jax.Array,
):
    return _build(A_x, A_k_cache, A_v_cache, A_wq, A_wo, B_w3, B_w4)
```

```python
import functools

import jax
import jax.numpy as jnp
from jax import lax
import jax.experimental.pallas as pl
import jax.experimental.pallas.tpu as pltpu

_F32 = jnp.float32
_BF16 = jnp.bfloat16
_L = 128
_EPS = 1e-5
_RING = 32


def _layernorm(x):
    m = jnp.mean(x, axis=-1, keepdims=True)
    c = x - m
    v = jnp.mean(c * c, axis=-1, keepdims=True)
    return c / jnp.sqrt(v + _EPS)


def _columns(row):
    return jnp.broadcast_to(row, (_L, _L)).T


def _perm(items, k):
    m = len(items) // k
    assert m * k == len(items)
    return [items[(i % k) * m + i // k] for i in range(len(items))]


class _Stream:
    def __init__(self, sems, priority, phase):
        self.sems, self.priority, self.n = sems, priority, phase
        self.pending = {}

    def adopt(self, slot, key, src, dst):
        self.pending[slot] = (key, pltpu.make_async_copy(src, dst, self.sems.at[slot]))

    def ensure(self, key):
        for slot, (k, _) in list(self.pending.items()):
            if k == key:
                self.wait_slot(slot)

    def wait_slot(self, slot):
        if slot in self.pending:
            self.pending.pop(slot)[1].wait()

    def start(self, key, src, dst):
        slot = self.n % _RING
        self.n += 1
        self.wait_slot(slot)
        cp = pltpu.make_async_copy(src, dst, self.sems.at[slot])
        cp.start(priority=self.priority)
        self.pending[slot] = (key, cp)

    def drain(self):
        for slot in list(self.pending):
            self.wait_slot(slot)


def _kernel(x_hbm, k_hbm, v_hbm, wq_hbm, wo_hbm, w3_hbm, w4_hbm, out_ref,
            xbuf, wqbuf, kbuf, vbuf, wobuf, w3buf, w4buf, qcol, slow, ssum, pb, xcol, qacc,
            sem_a, sem_b, *, H, DH, W, DA, W4E, W4LS, PACE):
    HD, SK = k_hbm.shape
    D, F = w3_hbm.shape
    PR = DH // 2
    NC = W // _L
    G = PR // 8
    DT = D // _L
    WS, WM = wq_hbm.shape[:2]
    assert NC == _RING and WM & (WM - 1) == 0 and wo_hbm.shape == wq_hbm.shape and WS % DT == 0

    def kv_piece(hbm, buf, row0, half, c):
        return hbm.at[pl.ds(row0, PR), pl.ds(SK - W + c * _L, _L)], buf.at[half, c]

    def q_rows(row0):
        return qcol[pl.ds(row0, PR), :]

    def softmax_p():
        s = ssum[pl.ds(0, NC, stride=8), :]
        for r in range(1, 8):
            s = s + ssum[pl.ds(r, NC, stride=8), :]
        s = s * (DH ** -0.5)
        m = jnp.max(jnp.max(s, axis=0, keepdims=True), axis=1, keepdims=True)
        e = jnp.exp(s - m)
        return e / jnp.sum(jnp.sum(e, axis=0, keepdims=True), axis=1, keepdims=True)

    def wo_mac(o, g, row0, att):
        if isinstance(row0, int):
            tiles = [wobuf[divmod((row0 // 8 + g) * DT + n, WM)] for n in range(DT)]
        else:
            t = (lax.shift_right_logical(row0, 3) + g) * DT
            tiles = [wobuf[lax.shift_right_logical(t + n, WM.bit_length() - 1), (t + n) & (WM - 1)]
                     for n in range(DT)]
        w = jnp.concatenate([tl.astype(_F32) for tl in tiles], axis=1)
        return att + w * jnp.broadcast_to(o[g * 8:(g + 1) * 8, :], (8, D))

    def half_slot(half, step, *, q=None, kslot=None, par=None, prev=None, att=None, p_out=None, extra=None):
        acc = None if par is None else jnp.zeros((PR, _L), _F32)
        o = p_new = None
        for c in range(NC):
            step(c)
            if c == 0 and prev is not None:
                o = jnp.sum(prev[0], axis=1, keepdims=True)
            if c == 0 and p_out is not None:
                p_new = softmax_p()
            if q is not None:
                part = jnp.sum((kbuf[1 - half if kslot is None else kslot, c].astype(_F32) * q).reshape(G, 8, _L), axis=0)
                if half == 0:
                    ssum[c * 8:(c + 1) * 8, :] = part + slow[c]
                else:
                    slow[c] = part
            if par is not None:
                vf = vbuf[half, c].astype(_F32).reshape(G, 8, _L)
                acc = acc + (vf * pb[par, c][None]).reshape(PR, _L)
            if prev is not None and 4 <= c < 4 + G:
                att = wo_mac(o, c - 4, prev[1], att)
            if p_out is not None and 8 <= c < 8 + NC // 2:
                for i in (2 * (c - 8), 2 * (c - 8) + 1):
                    pb[p_out, i] = jnp.broadcast_to(p_new[i:i + 1, :], (8, _L))
            if extra is not None:
                extra(c)
        return acc, att

    QW = 2 * _L

    def w_piece(key, hbm, buf, t, s0=0, s1=WS):
        return key, hbm.at[s0:s1, t], buf.at[s0:s1, t]

    k_p = [[(None,) + kv_piece(k_hbm, kbuf, hh * PR, sl, c) for c in range(NC)]
           for hh, sl in enumerate((2, 1, 0, 1))]
    v_p = [(None,) + kv_piece(v_hbm, vbuf, 0, 0, c) for c in range(NC)]
    n1 = WM - 3 * NC
    n2 = WM - (NC - DA)
    SH = WS // 2
    a_list = ([("x", x_hbm, xbuf)] + k_p[0] + k_p[1] + k_p[2]
              + [w_piece(None, wo_hbm, wobuf, t, 0, WS if t < n1 else SH) for t in range(n2)] + k_p[3])
    b_list = ([w_piece(None, wq_hbm, wqbuf, t) for t in range(WM)]
              + [w_piece(None, wo_hbm, wobuf, t, SH if t < n2 else 0, WS) for t in range(n1, WM)] + v_p)
    T0 = len(b_list) - NC
    up_a = len(a_list) - T0
    A = _Stream(sem_a, 0, -len(a_list) % _RING)
    B = _Stream(sem_b, 1, -len(b_list) % _RING)
    for pc in a_list[:up_a]:
        A.start(*pc)
    for pc in b_list[:_RING]:
        B.start(*pc)

    A.ensure("x")
    x = xbuf[...].astype(_F32)
    xn = _layernorm(x).astype(_BF16).astype(_F32)
    for j in range(DT):
        xcol[j] = _columns(xn[:, j * _L:(j + 1) * _L]).reshape(_L // 8, 8, _L)

    touched = set()

    def q_mac(t):
        w = wqbuf[:, t].astype(_F32).reshape(DT, WS // DT, 8, _L)
        for i in range(WS // DT):
            rt, ct = divmod(i * WM + t, HD // _L)
            term = jnp.sum(w[:, i] * xcol[:, rt], axis=0)
            cols = slice(ct * _L, (ct + 1) * _L)
            qacc[:, cols] = qacc[:, cols] + term if ct in touched else term
            touched.add(ct)

    def q_fin(r0):
        q = jnp.sum(qacc[:, pl.ds(r0, QW)], axis=0, keepdims=True).astype(_BF16).astype(_F32)
        for j in range(0, QW, _L):
            qcol[pl.ds(r0 + j, _L), :] = _columns(q[:, j:j + _L])

    t_k = T0 - 3 * NC
    NQP = 3
    assert t_k == WM

    def pre_step(t):
        B.wait_slot(B.n % _RING)
        A.start(*a_list[up_a + t])
        B.start(*b_list[t + _RING])

    for t in range(t_k):
        pre_step(t)
        q_mac(t)
    q_fin(0)
    half_slot(1, lambda c: pre_step(t_k + c), q=q_rows(0), kslot=2)
    half_slot(0, lambda c: pre_step(t_k + NC + c), q=q_rows(PR), extra=lambda c: q_fin(QW) if c == 0 else None)
    half_slot(1, lambda c: pre_step(t_k + 2 * NC + c), q=q_rows(DH), p_out=0,
              extra=lambda c: q_fin(2 * QW) if c == 0 else None)

    def loop_step(j, half):
        r_k = pl.multiple_of((j + 2) * DH + half * PR, 8)
        r_v = pl.multiple_of(j * DH + (half + 1) * PR, 8)

        def step(c):
            pltpu.make_async_copy(*kv_piece(v_hbm, vbuf, 0, half, c), sem_b.at[c]).wait()
            pltpu.make_async_copy(*kv_piece(k_hbm, kbuf, 0, 1 - half, c), sem_a.at[c]).wait()
            pltpu.make_async_copy(*kv_piece(k_hbm, kbuf, r_k, half, c), sem_a.at[c]).start(priority=0)
            pltpu.make_async_copy(*kv_piece(v_hbm, vbuf, r_v, 1 - half, c), sem_b.at[c]).start(priority=1)
        return step

    def head(j, carry):
        acc, att = carry
        par = j & 1
        r0 = pl.multiple_of(j * DH, 8)
        r_q = pl.multiple_of(jnp.minimum((NQP + j) * QW, HD - QW), _L)
        acc, att = half_slot(0, loop_step(j, 0), q=q_rows(r0 + DH + PR), par=par,
                             prev=(acc, jnp.maximum(r0 - PR, 0)), att=att)
        return half_slot(1, loop_step(j, 1), q=q_rows(r0 + 2 * DH), par=par, prev=(acc, r0), att=att,
                         p_out=1 - par, extra=lambda c: q_fin(r_q) if c == 0 else None)

    NL = H - 2
    acc, att = lax.fori_loop(0, NL, head, (jnp.zeros((PR, _L), _F32), jnp.zeros((8, D), _F32)))

    A = _Stream(sem_a, 0, 0)
    B = _Stream(sem_b, 1, 0)
    for c in range(NC):
        A.adopt(c, ("k", c), *kv_piece(k_hbm, kbuf, 0, 1, c))
        B.adopt(c, None, *kv_piece(v_hbm, vbuf, 0, 0, c))

    def rows(key, hbm, buf, r0, r1, n):
        return [(key or r, hbm.at[pl.ds(r, n), :], buf.at[pl.ds(r, n), :]) for r in range(r0, r1, n)]

    RE = W4E * _L
    a_early = _perm(rows("w", w3_hbm, w3buf, 0, D, 8), 4) + _perm(rows("w", w4_hbm, w4buf, 0, RE, 16), 2)
    w4_late = _perm(rows(None, w4_hbm, w4buf, RE, F, W4LS), 2)
    late_a = w4_late[1:2 * sum(PACE):2]
    b_post = ([(None,) + kv_piece(v_hbm, vbuf, hh * PR, hh % 2, c)
               for hh in range(2 * NL + 1, 2 * H) for c in range(NC)]
              + [pc for pc in w4_late if not any(pc is o for o in late_a)])
    assert len(b_post) <= 4 * NC and len(a_early) <= 4 * NC
    a_sched = {(i * 4 * NC) // len(a_early): pc for i, pc in enumerate(a_early)}

    def post_step(t):
        B.wait_slot(t % _RING)
        A.ensure(("k", t))
        if t in a_sched:
            A.start(*a_sched[t])
        if t < len(b_post):
            B.start(*b_post[t])

    r0, par = NL * DH, NL & 1
    acc, att = half_slot(0, post_step, q=q_rows(r0 + DH + PR), par=par, prev=(acc, r0 - PR), att=att)
    acc, att = half_slot(1, lambda c: post_step(NC + c), par=par, prev=(acc, r0), att=att, p_out=1 - par)
    acc, att = half_slot(0, lambda c: post_step(2 * NC + c), par=1 - par, prev=(acc, r0 + PR), att=att)
    acc, att = half_slot(1, lambda c: post_step(3 * NC + c), par=1 - par, prev=(acc, r0 + DH), att=att)

    o = jnp.sum(acc, axis=1, keepdims=True)
    for g in range(G):
        att = wo_mac(o, g, r0 + DH + PR, att)
    for pc in late_a[:PACE[0]]:
        A.start(*pc)
    hres = x + jnp.sum(att, axis=0, keepdims=True)
    x1 = _layernorm(hres)
    y = jnp.broadcast_to(_layernorm(x1).astype(_BF16), (8, D))
    for pc in late_a[PACE[0]:]:
        A.start(*pc)
    A.ensure("w")
    hid = jax.nn.gelu(jnp.dot(y, w3buf[...], preferred_element_type=_F32), approximate=True).astype(_BF16)
    res = hres + x1 + jnp.dot(hid[:, :RE], w4buf[:RE, :], preferred_element_type=_F32)[0:1, :]
    hrow = hid[0:1, :].astype(_F32)
    for r in range(RE, F, _L):
        qcol[r:r + _L, :] = _columns(hrow[:, r:r + _L])
    tail = jnp.zeros((8, D), _F32)
    for r, _, _ in w4_late:
        A.ensure(r)
        B.ensure(r)
        for rr in range(r, r + W4LS, 8):
            hc = jnp.concatenate([qcol[rr:rr + 8, :]] * (D // _L), axis=1)
            tail = tail + w4buf[rr:rr + 8, :].astype(_F32) * hc
    A.drain()
    B.drain()
    out_ref[...] = (res + jnp.sum(tail, axis=0, keepdims=True)).astype(out_ref.dtype)


def _tile_streams(w):
    r, c = w.shape
    return w.reshape(r // 8, 8, c // _L, _L).transpose(0, 2, 1, 3).reshape(-1, 256, 8, _L)


def _compiler_params():
    base = dict(vmem_limit_bytes=48 * 1024 * 1024)
    try:
        return pltpu.CompilerParams(disable_bounds_checks=True, disable_semaphore_checks=True, **base)
    except TypeError:
        return pltpu.CompilerParams(**base)


def _build(A_x, A_k_cache, A_v_cache, A_wq, A_wo, B_w3, B_w4, *, DA=12, W4E=4, W4LS=32, PACE=(3, 4)):
    B, S, D = A_x.shape
    _, H, SK, DH = A_k_cache.shape
    assert B == 1 and S == 1
    W = min(4096, max(256, SK // 4))
    HD = H * DH
    NC = W // _L
    kt = jnp.swapaxes(A_k_cache[0], 1, 2).reshape(HD, SK)
    vt = jnp.swapaxes(A_v_cache[0], 1, 2).reshape(HD, SK)
    wq4 = _tile_streams(A_wq)
    wo4 = _tile_streams(A_wo)
    out = pl.pallas_call(
        functools.partial(_kernel, H=H, DH=DH, W=W, DA=DA, W4E=W4E, W4LS=W4LS, PACE=PACE),
        out_shape=jax.ShapeDtypeStruct((1, D), A_x.dtype),
        in_specs=[pl.BlockSpec(memory_space=pl.ANY)] * 7,
        out_specs=pl.BlockSpec(memory_space=pltpu.VMEM),
        scratch_shapes=[
            pltpu.VMEM((1, D), A_x.dtype),
            pltpu.VMEM(wq4.shape, A_wq.dtype),
            pltpu.VMEM((3, NC, DH // 2, _L), A_k_cache.dtype),
            pltpu.VMEM((2, NC, DH // 2, _L), A_v_cache.dtype),
            pltpu.VMEM(wo4.shape, A_wo.dtype),
            pltpu.VMEM(B_w3.shape, B_w3.dtype),
            pltpu.VMEM(B_w4.shape, B_w4.dtype),
            pltpu.VMEM((HD, _L), _F32),
            pltpu.VMEM((NC, 8, _L), _F32),
            pltpu.VMEM((NC * 8, _L), _F32),
            pltpu.VMEM((2, NC, 8, _L), _F32),
            pltpu.VMEM((D // _L, _L // 8, 8, _L), _F32),
            pltpu.VMEM((8, HD), _F32),
            pltpu.SemaphoreType.DMA((_RING,)),
            pltpu.SemaphoreType.DMA((_RING,)),
        ],
        compiler_params=_compiler_params(),
    )(A_x.reshape(1, D), kt, vt, wq4, wo4, B_w3, B_w4)
    return out.reshape(B, S, D)


@jax.jit
def pallas_sequential_preLN__sliding_block_cached__mixer_s_mlp__decode_kernel(
    A_x: jax.Array,
    A_k_cache: jax.Array,
    A_v_cache: jax.Array,
    A_wq: jax.Array,
    A_wo: jax.Array,
    B_x: jax.Array,
    B_w1: jax.Array,
    B_w2: jax.Array,
    B_w3: jax.Array,
    B_w4: jax.Array,
):
    return _build(A_x, A_k_cache, A_v_cache, A_wq, A_wo, B_w3, B_w4)
```

```python
import functools

import jax
import jax.numpy as jnp
from jax import lax
import jax.experimental.pallas as pl
import jax.experimental.pallas.tpu as pltpu

_F32 = jnp.float32
_BF16 = jnp.bfloat16
_L = 128
_EPS = 1e-5
_RING = 32


def _layernorm(x):
    m = jnp.mean(x, axis=-1, keepdims=True)
    c = x - m
    v = jnp.mean(c * c, axis=-1, keepdims=True)
    return c / jnp.sqrt(v + _EPS)


def _columns(row):
    return jnp.broadcast_to(row, (_L, _L)).T


def _perm(items, k):
    m = len(items) // k
    assert m * k == len(items)
    return [items[(i % k) * m + i // k] for i in range(len(items))]


class _Stream:
    def __init__(self, sems, priority, phase):
        self.sems, self.priority, self.n = sems, priority, phase
        self.pending = {}

    def adopt(self, slot, key, src, dst):
        self.pending[slot] = (key, pltpu.make_async_copy(src, dst, self.sems.at[slot]))

    def ensure(self, key):
        for slot, (k, _) in list(self.pending.items()):
            if k == key:
                self.wait_slot(slot)

    def wait_slot(self, slot):
        if slot in self.pending:
            self.pending.pop(slot)[1].wait()

    def start(self, key, src, dst):
        slot = self.n % _RING
        self.n += 1
        self.wait_slot(slot)
        cp = pltpu.make_async_copy(src, dst, self.sems.at[slot])
        cp.start(priority=self.priority)
        self.pending[slot] = (key, cp)

    def drain(self):
        for slot in list(self.pending):
            self.wait_slot(slot)


def _kernel(x_hbm, k_hbm, v_hbm, wq_hbm, wo_hbm, w3_hbm, w4_hbm, out_ref,
            xbuf, wqbuf, kbuf, vbuf, wobuf, w3buf, w4buf, qcol, slow, ssum, pb, xcol, qacc,
            sem_a, sem_b, *, H, DH, W, DA, W4E, W4LS, PACE):
    HD, SK = k_hbm.shape
    D, F = w3_hbm.shape
    PR = DH // 2
    NC = W // _L
    G = PR // 8
    DT = D // _L
    WS, WM = wq_hbm.shape[:2]
    assert NC == _RING and WM & (WM - 1) == 0 and wo_hbm.shape == wq_hbm.shape and WS % DT == 0

    def kv_piece(hbm, buf, row0, half, c):
        return hbm.at[pl.ds(row0, PR), pl.ds(SK - W + c * _L, _L)], buf.at[half, c]

    def q_rows(row0):
        return qcol[pl.ds(row0, PR), :]

    def softmax_p():
        s = ssum[pl.ds(0, NC, stride=8), :]
        for r in range(1, 8):
            s = s + ssum[pl.ds(r, NC, stride=8), :]
        s = s * (DH ** -0.5)
        m = jnp.max(jnp.max(s, axis=0, keepdims=True), axis=1, keepdims=True)
        e = jnp.exp(s - m)
        return e / jnp.sum(jnp.sum(e, axis=0, keepdims=True), axis=1, keepdims=True)

    def wo_mac(o, g, row0, att):
        if isinstance(row0, int):
            tiles = [wobuf[divmod((row0 // 8 + g) * DT + n, WM)] for n in range(DT)]
        else:
            t = (lax.shift_right_logical(row0, 3) + g) * DT
            tiles = [wobuf[lax.shift_right_logical(t + n, WM.bit_length() - 1), (t + n) & (WM - 1)]
                     for n in range(DT)]
        w = jnp.concatenate([tl.astype(_F32) for tl in tiles], axis=1)
        return att + w * jnp.broadcast_to(o[g * 8:(g + 1) * 8, :], (8, D))

    def half_slot(half, step, *, q=None, kslot=None, par=None, prev=None, att=None, p_out=None, extra=None):
        acc = None if par is None else jnp.zeros((PR, _L), _F32)
        o = p_new = None
        for c in range(NC):
            step(c)
            if c == 0 and prev is not None:
                o = jnp.sum(prev[0], axis=1, keepdims=True)
            if c == 0 and p_out is not None:
                p_new = softmax_p()
            if q is not None:
                kf = kbuf[1 - half if kslot is None else kslot, c].astype(_F32)
                part = jnp.sum((kf * q).reshape(G, 8, _L), axis=0)
                if half == 0:
                    ssum[c * 8:(c + 1) * 8, :] = part + slow[c]
                else:
                    slow[c] = part
            if par is not None:
                vf = vbuf[half, c].astype(_F32).reshape(G, 8, _L)
                acc = acc + (vf * pb[par, c][None]).reshape(PR, _L)
            if prev is not None and 4 <= c < 4 + G:
                att = wo_mac(o, c - 4, prev[1], att)
            if p_out is not None and 8 <= c < 8 + NC // 2:
                for i in (2 * (c - 8), 2 * (c - 8) + 1):
                    pb[p_out, i] = jnp.broadcast_to(p_new[i:i + 1, :], (8, _L))
            if extra is not None:
                extra(c)
        return acc, att

    QW = 2 * _L

    def w_piece(hbm, buf, t, s0=0, s1=WS):
        return None, hbm.at[s0:s1, t], buf.at[s0:s1, t]

    k_p = [[(None,) + kv_piece(k_hbm, kbuf, hh * PR, sl, c) for c in range(NC)]
           for hh, sl in enumerate((2, 1, 0, 1))]
    v_p = [(None,) + kv_piece(v_hbm, vbuf, 0, 0, c) for c in range(NC)]
    n1 = WM - 3 * NC
    n2 = WM - (NC - DA)
    SH = WS // 2
    a_list = ([("x", x_hbm, xbuf)] + k_p[0] + k_p[1] + k_p[2]
              + [w_piece(wo_hbm, wobuf, t, 0, WS if t < n1 else SH) for t in range(n2)] + k_p[3])
    b_list = ([w_piece(wq_hbm, wqbuf, t) for t in range(WM)]
              + [w_piece(wo_hbm, wobuf, t, SH if t < n2 else 0, WS) for t in range(n1, WM)] + v_p)
    T0 = len(b_list) - NC
    up_a = len(a_list) - T0
    A = _Stream(sem_a, 0, -len(a_list) % _RING)
    B = _Stream(sem_b, 1, -len(b_list) % _RING)
    for pc in a_list[:up_a]:
        A.start(*pc)
    for pc in b_list[:_RING]:
        B.start(*pc)

    A.ensure("x")
    x = xbuf[...].astype(_F32)
    xn = _layernorm(x).astype(_BF16).astype(_F32)
    for j in range(DT):
        xcol[j] = _columns(xn[:, j * _L:(j + 1) * _L]).reshape(_L // 8, 8, _L)

    touched = set()

    def q_mac(t):
        w = wqbuf[:, t].astype(_F32).reshape(DT, WS // DT, 8, _L)
        for i in range(WS // DT):
            rt, ct = divmod(i * WM + t, HD // _L)
            term = jnp.sum(w[:, i] * xcol[:, rt], axis=0)
            cols = slice(ct * _L, (ct + 1) * _L)
            qacc[:, cols] = qacc[:, cols] + term if ct in touched else term
            touched.add(ct)

    def q_fin(r0):
        q = jnp.sum(qacc[:, pl.ds(r0, QW)], axis=0, keepdims=True).astype(_BF16).astype(_F32)
        for j in range(0, QW, _L):
            qcol[pl.ds(r0 + j, _L), :] = _columns(q[:, j:j + _L])

    t_k = T0 - 3 * NC
    NQP = 3
    assert t_k == WM

    def pre_step(t):
        B.wait_slot(B.n % _RING)
        A.start(*a_list[up_a + t])
        B.start(*b_list[t + _RING])

    for t in range(t_k):
        pre_step(t)
        q_mac(t)
    q_fin(0)
    half_slot(1, lambda c: pre_step(t_k + c), q=q_rows(0), kslot=2)
    half_slot(0, lambda c: pre_step(t_k + NC + c), q=q_rows(PR), extra=lambda c: q_fin(QW) if c == 0 else None)
    half_slot(1, lambda c: pre_step(t_k + 2 * NC + c), q=q_rows(DH), p_out=0,
              extra=lambda c: q_fin(2 * QW) if c == 0 else None)

    def loop_step(j, half):
        r_k = pl.multiple_of((j + 2) * DH + half * PR, 8)
        r_v = pl.multiple_of(j * DH + (half + 1) * PR, 8)
        r_kw = pl.multiple_of(r_k - PR, 8)
        r_vw = pl.multiple_of(r_v - PR, 8)

        def step(c):
            pltpu.make_async_copy(*kv_piece(v_hbm, vbuf, r_vw, half, c), sem_b.at[c]).wait()
            pltpu.make_async_copy(*kv_piece(k_hbm, kbuf, r_kw, 1 - half, c), sem_a.at[c]).wait()
            pltpu.make_async_copy(*kv_piece(k_hbm, kbuf, r_k, half, c), sem_a.at[c]).start(priority=0)
            pltpu.make_async_copy(*kv_piece(v_hbm, vbuf, r_v, 1 - half, c), sem_b.at[c]).start(priority=1)
        return step

    def head(j, carry):
        acc, att = carry
        par = j & 1
        r0 = pl.multiple_of(j * DH, 8)
        r_q = pl.multiple_of(jnp.minimum((NQP + j) * QW, HD - QW), _L)
        acc, att = half_slot(0, loop_step(j, 0), q=q_rows(r0 + DH + PR), par=par,
                             prev=(acc, jnp.maximum(r0 - PR, 0)), att=att)
        return half_slot(1, loop_step(j, 1), q=q_rows(r0 + 2 * DH), par=par, prev=(acc, r0), att=att,
                         p_out=1 - par, extra=lambda c: q_fin(r_q) if c == 0 else None)

    NL = H - 2
    acc, att = lax.fori_loop(0, NL, head, (jnp.zeros((PR, _L), _F32), jnp.zeros((8, D), _F32)))

    A = _Stream(sem_a, 0, 0)
    B = _Stream(sem_b, 1, 0)
    for c in range(NC):
        A.adopt(c, ("k", c), *kv_piece(k_hbm, kbuf, HD - PR, 1, c))
        B.adopt(c, None, *kv_piece(v_hbm, vbuf, NL * DH, 0, c))

    def rows(key, hbm, buf, r0, r1, n):
        return [(key or r, hbm.at[pl.ds(r, n), :], buf.at[pl.ds(r, n), :]) for r in range(r0, r1, n)]

    RE = W4E * _L
    a_early = _perm(rows("w", w3_hbm, w3buf, 0, D, 8), 4) + _perm(rows("w", w4_hbm, w4buf, 0, RE, 16), 2)
    w4_late = _perm(rows(None, w4_hbm, w4buf, RE, F, W4LS), 2)
    late_a = w4_late[1:2 * sum(PACE):2]
    b_post = ([(None,) + kv_piece(v_hbm, vbuf, hh * PR, hh % 2, c)
               for hh in range(2 * NL + 1, 2 * H) for c in range(NC)]
              + [pc for pc in w4_late if not any(pc is o for o in late_a)])
    assert len(b_post) <= 4 * NC and len(a_early) <= 4 * NC
    a_sched = {(i * 4 * NC) // len(a_early): pc for i, pc in enumerate(a_early)}

    def post_step(t):
        B.wait_slot(t % _RING)
        A.ensure(("k", t))
        if t in a_sched:
            A.start(*a_sched[t])
        if t < len(b_post):
            B.start(*b_post[t])

    r0, par = NL * DH, NL & 1
    acc, att = half_slot(0, post_step, q=q_rows(r0 + DH + PR), par=par, prev=(acc, r0 - PR), att=att)
    acc, att = half_slot(1, lambda c: post_step(NC + c), par=par, prev=(acc, r0), att=att, p_out=1 - par)
    acc, att = half_slot(0, lambda c: post_step(2 * NC + c), par=1 - par, prev=(acc, r0 + PR), att=att)
    acc, att = half_slot(1, lambda c: post_step(3 * NC + c), par=1 - par, prev=(acc, r0 + DH), att=att)

    o = jnp.sum(acc, axis=1, keepdims=True)
    for g in range(G):
        att = wo_mac(o, g, r0 + DH + PR, att)
    for pc in late_a[:PACE[0]]:
        A.start(*pc)
    hres = x + jnp.sum(att, axis=0, keepdims=True)
    x1 = _layernorm(hres)
    y = jnp.broadcast_to(_layernorm(x1).astype(_BF16), (8, D))
    for pc in late_a[PACE[0]:]:
        A.start(*pc)
    A.ensure("w")
    hid = jax.nn.gelu(jnp.dot(y, w3buf[...], preferred_element_type=_F32), approximate=True).astype(_BF16)
    res = hres + x1 + jnp.dot(hid[:, :RE], w4buf[:RE, :], preferred_element_type=_F32)[0:1, :]
    hrow = hid[0:1, :].astype(_F32)
    for r in range(RE, F, _L):
        qcol[r:r + _L, :] = _columns(hrow[:, r:r + _L])
    tail = jnp.zeros((8, D), _F32)
    for r, _, _ in w4_late:
        A.ensure(r)
        B.ensure(r)
        for rr in range(r, r + W4LS, 8):
            hc = jnp.concatenate([qcol[rr:rr + 8, :]] * (D // _L), axis=1)
            tail = tail + w4buf[rr:rr + 8, :].astype(_F32) * hc
    A.drain()
    B.drain()
    out_ref[...] = (res + jnp.sum(tail, axis=0, keepdims=True)).astype(out_ref.dtype)


def _tile_streams(w):
    r, c = w.shape
    return w.reshape(r // 8, 8, c // _L, _L).transpose(0, 2, 1, 3).reshape(-1, 256, 8, _L)


def _compiler_params():
    base = dict(vmem_limit_bytes=48 * 1024 * 1024)
    try:
        return pltpu.CompilerParams(disable_bounds_checks=True, disable_semaphore_checks=True, **base)
    except TypeError:
        return pltpu.CompilerParams(**base)


def _build(A_x, A_k_cache, A_v_cache, A_wq, A_wo, B_w3, B_w4, *, DA=12, W4E=4, W4LS=32, PACE=(3, 4)):
    B, S, D = A_x.shape
    _, H, SK, DH = A_k_cache.shape
    assert B == 1 and S == 1
    W = min(4096, max(256, SK // 4))
    HD = H * DH
    NC = W // _L
    kt = jnp.swapaxes(A_k_cache[0], 1, 2).reshape(HD, SK)
    vt = jnp.swapaxes(A_v_cache[0], 1, 2).reshape(HD, SK)
    wq4 = _tile_streams(A_wq)
    wo4 = _tile_streams(A_wo)
    out = pl.pallas_call(
        functools.partial(_kernel, H=H, DH=DH, W=W, DA=DA, W4E=W4E, W4LS=W4LS, PACE=PACE),
        out_shape=jax.ShapeDtypeStruct((1, D), A_x.dtype),
        in_specs=[pl.BlockSpec(memory_space=pl.ANY)] * 7,
        out_specs=pl.BlockSpec(memory_space=pltpu.VMEM),
        scratch_shapes=[
            pltpu.VMEM((1, D), A_x.dtype),
            pltpu.VMEM(wq4.shape, A_wq.dtype),
            pltpu.VMEM((3, NC, DH // 2, _L), A_k_cache.dtype),
            pltpu.VMEM((2, NC, DH // 2, _L), A_v_cache.dtype),
            pltpu.VMEM(wo4.shape, A_wo.dtype),
            pltpu.VMEM(B_w3.shape, B_w3.dtype),
            pltpu.VMEM(B_w4.shape, B_w4.dtype),
            pltpu.VMEM((HD, _L), _F32),
            pltpu.VMEM((NC, 8, _L), _F32),
            pltpu.VMEM((NC * 8, _L), _F32),
            pltpu.VMEM((2, NC, 8, _L), _F32),
            pltpu.VMEM((D // _L, _L // 8, 8, _L), _F32),
            pltpu.VMEM((8, HD), _F32),
            pltpu.SemaphoreType.DMA((_RING,)),
            pltpu.SemaphoreType.DMA((_RING,)),
        ],
        compiler_params=_compiler_params(),
    )(A_x.reshape(1, D), kt, vt, wq4, wo4, B_w3, B_w4)
    return out.reshape(B, S, D)


@jax.jit
def pallas_sequential_preLN__sliding_block_cached__mixer_s_mlp__decode_kernel(
    A_x: jax.Array,
    A_k_cache: jax.Array,
    A_v_cache: jax.Array,
    A_wq: jax.Array,
    A_wo: jax.Array,
    B_x: jax.Array,
    B_w1: jax.Array,
    B_w2: jax.Array,
    B_w3: jax.Array,
    B_w4: jax.Array,
):
    return _build(A_x, A_k_cache, A_v_cache, A_wq, A_wo, B_w3, B_w4)
```
